```python
import os as _os
_os.environ.setdefault('JAX_PLATFORMS', 'cpu')
import jax
import jax.numpy as jnp

def _softmax(x, axis=-1):
    return jax.nn.softmax(x, axis=axis)

def _gelu(x):
    return jax.nn.gelu(x, approximate=True)

def _silu(x):
    return jax.nn.silu(x)

def _sigmoid(x):
    return jax.nn.sigmoid(x)

def _layernorm(x, axis=-1, eps=1e-05):
    m = jnp.mean(x, axis=axis, keepdims=True)
    v = jnp.var(x, axis=axis, keepdims=True)
    return (x - m) / jnp.sqrt(v + eps)

def _scatter_add(tgt, idx, src, axis=0):
    return tgt.at[idx].add(src)

def _segment_sum(src, seg, n):
    return jax.ops.segment_sum(src, seg, n)

class _Rng:

    def __init__(self, key):
        self._k = key

    def _next(self):
        self._k, sub = jax.random.split(self._k)
        return sub

    def normal(self, shape):
        return jax.random.normal(self._next(), shape, dtype=jnp.bfloat16)

    def randint(self, lo, hi, shape):
        return jax.random.randint(self._next(), shape, lo, hi, dtype=jnp.int32)

    def uniform(self, shape, lo=0.0, hi=1.0):
        return jax.random.uniform(self._next(), shape, jnp.bfloat16, lo, hi)

    def permutation(self, n):
        return jax.random.permutation(self._next(), n)
kernel_name = 'parallel_sum__memory_aug_recurrent_mem_tr__dense_activation_silu__prompt'

def setup_inputs():
    _rng = _Rng(jax.random.key(int.from_bytes(__import__("os").urandom(4), "little")))
    _w = lambda a: (lambda t: t.astype(jnp.bfloat16) if jnp.issubdtype(t.dtype, jnp.floating) else t)(jnp.asarray(a))

    def _A_setup():
        B, S, Dm = (1, 2048, 448)
        H, Dh = (16, 256)
        M, seg = (8, 32)
        seg = min(seg, S)
        S = S // seg * seg
        return {'x': _w((lambda *s: _rng.normal(s) * 0.05)(B, S, Dm)), 'mem0': _w((lambda *s: _rng.normal(s) * 0.2)(B, M, Dm)), 'Wq': _w((lambda *s: _rng.normal(s) * 0.8)(Dm, H, Dh) * Dm ** (-0.5)), 'Wk': _w((lambda *s: _rng.normal(s) * 0.8)(Dm, H, Dh) * Dm ** (-0.5)), 'Wv': _w((lambda *s: _rng.normal(s) * 0.2)(Dm, H, Dh) * Dm ** (-0.5)), 'Wo': _w((lambda *s: _rng.normal(s) * 0.2)(H, Dh, Dm) * (H * Dh) ** (-0.5)), 'seg_len': seg}
    _A_in = _A_setup()

    def _B_setup():
        B, S, D, F = (1, 2048, 448, 1792)
        return {'x': _w((lambda *s: _rng.normal(s) * 0.05)(B, S, D)), 'w1': _w((lambda *s: _rng.normal(s) * 0.05)(D, F) * D ** (-0.5)), 'w2': _w((lambda *s: _rng.normal(s) * 0.05)(F, D) * F ** (-0.5))}
    _B_in = _B_setup()
    return {'A_x': _A_in['x'], 'A_mem0': _A_in['mem0'], 'A_Wq': _A_in['Wq'], 'A_Wk': _A_in['Wk'], 'A_Wv': _A_in['Wv'], 'A_Wo': _A_in['Wo'], 'A_seg_len': _A_in['seg_len'], 'B_x': _B_in['x'], 'B_w1': _B_in['w1'], 'B_w2': _B_in['w2']}

def reference(A_x, A_mem0, A_Wq, A_Wk, A_Wv, A_Wo, A_seg_len, B_x, B_w1, B_w2):

    def _A_ref(x, mem0, Wq, Wk, Wv, Wo, seg_len):
        B, S, Dm = x.shape
        H, Dh = (Wq.shape[1], Wq.shape[2])
        M = mem0.shape[1]
        scale = Dh ** (-0.5)
        n_seg = S // seg_len
        L = M + seg_len
        idx = jnp.arange(L)
        mask = (idx[:, None] < M) | (idx[:, None] >= idx[None, :])
        mem = mem0
        outs = []
        for s in range(n_seg):
            xs = x[:, s * seg_len:(s + 1) * seg_len, :].copy()
            h = jnp.concatenate([mem, xs], axis=1)
            q = jnp.einsum('btd,dhe->bhte', h, Wq)
            k = jnp.einsum('btd,dhe->bhte', h, Wk)
            v = jnp.einsum('btd,dhe->bhte', h, Wv)
            scores = jnp.einsum('bhqe,bhke->bhqk', q, k) * scale
            scores = jnp.where(mask[None, None], scores, -1000000000.0)
            p = _softmax(scores, axis=-1)
            o = jnp.einsum('bhqk,bhke->bhqe', p, v)
            o = jnp.einsum('bhte,hed->btd', o, Wo)
            mem = o[:, :M, :].copy()
            outs.append(o[:, M:, :])
        return jnp.concatenate(outs, axis=1)

    def _B_ref(x, w1, w2):
        h = jnp.einsum('bsd,df->bsf', x, w1)
        h = _silu(h)
        out = jnp.einsum('bsf,fd->bsd', h, w2)
        return out
    x = A_x
    xn = _layernorm(x, axis=-1)
    return x + _A_ref(xn, A_mem0, A_Wq, A_Wk, A_Wv, A_Wo, A_seg_len) + _B_ref(xn, B_w1, B_w2)
```

```python
import jax
import jax.numpy as jnp
import numpy as np
from jax.experimental import pallas as pl
from jax.experimental.pallas import tpu as pltpu

S, D, H, DH, M, SEG, F = 2048, 448, 16, 256, 8, 32, 1792
NSEG = S // SEG
L = M + SEG
DP = 512
UNROLL = 4
NBLK = S // 128
f32, bf16, u32 = jnp.float32, jnp.bfloat16, jnp.uint32
NT = (((1,), (1,)), ((), ()))
NN = (((1,), (0,)), ((), ()))
XT = True
NU0 = 3


def _dot(a, b, dims=NN):
    return jax.lax.dot_general(a, b, dims, preferred_element_type=f32)


def _pack(x):
    return pltpu.bitcast(x.astype(bf16), u32)


def _unpack(x):
    return pltpu.bitcast(x, bf16)


_PARTS = [[(j, max(40 * j, 128 * t) - 128 * t, min(40 * j + 40, 128 * t + 128) - 128 * t)
           for j in range(H) if 40 * j < 128 * t + 128 and 40 * j + 40 > 128 * t] for t in range(5)]


def kernel(x_hbm, mem_ref, wq_hbm, wk_hbm, wv_hbm, wo_hbm, w1_hbm, w2_hbm, out_hbm,
           q_scr, k_scr, v_scr, wo_scr, x_scr, w1_raw, w2_raw, sems, osems,
           w_scr, xn_scr, w1_scr, w2_scr, res_scr, out_scr, hid_scr, tt_scr):
    def halves(src, dst, s0):
        return [pltpu.make_async_copy(src.at[:, pl.ds(c * 128, 128)], dst.at[c], sems.at[s0 + c]) for c in range(2)]
    cq, ck, cv = halves(wq_hbm, q_scr, 0), halves(wk_hbm, k_scr, 2), halves(wv_hbm, v_scr, 4)
    co = pltpu.make_async_copy(wo_hbm, wo_scr, sems.at[6])
    cx = pltpu.make_async_copy(x_hbm, x_scr, sems.at[7])
    c1 = pltpu.make_async_copy(w1_hbm, w1_raw, sems.at[8])
    c2 = pltpu.make_async_copy(w2_hbm, w2_raw, sems.at[9])
    for c in cq + ck:
        c.start()
    for c in cq + ck:
        c.wait()
    for c in cv + [co, cx]:
        c.start()

    def get(scr, p):
        los, his = [], []
        for c in range(2):
            x = scr.at[c].bitcast(u32)[pl.ds(p, D, stride=8), :]
            los.append(pltpu.bitcast(x << 16, f32))
            his.append(pltpu.bitcast(x & jnp.uint32(0xffff0000), f32))
        return jnp.concatenate(los, axis=1), jnp.concatenate(his, axis=1)

    def put(idx, e, o):
        w_scr[idx, 0:D // 2, 0:384] = _pack(e[:, :384])
        w_scr[idx, 0:D // 2, 384:768] = _pack(o[:, :384])
        w_scr[idx, 0:D // 2, 768:896] = _pack(jnp.concatenate([e[:, 384:448], o[:, 384:448]], axis=1))
        w_scr[idx, D // 2:DP // 2, :] = jnp.zeros(((DP - D) // 2, 896), u32)

    scale = DH ** -0.5
    for p in range(8):
        qlo, qhi = get(q_scr, p)
        klo, khi = get(k_scr, p)
        put(p, _dot(klo, qlo, NT) * scale, _dot(khi, qhi, NT) * scale)

    c1.start()
    c2.start()
    for c in cv + [co, cx]:
        c.wait()

    def layernorm(j):
        xb = x_scr[:, j * 128:(j + 1) * 128].astype(f32)
        mu = jnp.mean(xb, axis=0, keepdims=True)
        xc = xb - mu
        var = jnp.mean(xc * xc, axis=0, keepdims=True)
        xn = (xc * jax.lax.rsqrt(var + 1e-5)).astype(bf16).astype(f32)
        xn = jnp.concatenate([xn, jnp.zeros((DP - D, 128), f32)], axis=0)
        xn_scr[j * 128:(j + 1) * 128, :] = xn.T

    for p in range(8):
        vlo, vhi = get(v_scr, p)
        put(p + 8, _dot(vlo, wo_scr[2 * p], NT), _dot(vhi, wo_scr[2 * p + 1], NT))
        layernorm(2 * p)
        layernorm(2 * p + 1)
        if p == 5:
            c1.wait()
            c2.wait()
        if p == 6:
            w1_scr[0:D // 2, :] = pltpu.bitcast(w1_raw[...], u32)
            w1_scr[D // 2:DP // 2, :] = jnp.zeros(((DP - D) // 2, F), u32)
        if p == 7:
            w2t = jnp.concatenate([w2_raw[...], jnp.zeros((DP - D, F), bf16)], axis=0)
            w2_scr[...] = pltpu.bitcast(w2t.T, u32)
    res_scr[...] = jnp.zeros((128, DP), f32)

    lane = jax.lax.broadcasted_iota(jnp.int32, (L, 128), 1)
    row = jax.lax.broadcasted_iota(jnp.int32, (L, 128), 0)
    low = lane < 64

    def proj(h, idx):
        return _dot(h, _unpack(w_scr[idx]))

    def stacks(pr):
        rows = []
        for r in pr:
            rem = r[:, 768:896]
            rows.append(jnp.concatenate([r[:, 0:384], jnp.where(low, rem, 0.0)], axis=1))
            rows.append(jnp.concatenate([r[:, 384:768], jnp.where(low, 0.0, rem)], axis=1))
        return jnp.concatenate(rows, axis=0).astype(bf16)

    def softmax(sc):
        sg, masks = [], []
        for t in range(5):
            col = lane + 128 * t
            key = col
            for (j, lo, hi) in _PARTS[t]:
                key = jnp.where(lane >= lo, col - 40 * j, key)
            valid = (row < M) | (row >= key)
            sg.append(jnp.where(valid, sc[:, t * 128:(t + 1) * 128], -1e9))
            masks.append([(lane >= lo) & (lane < hi) for (_, lo, hi) in _PARTS[t]])

        def reduce(vals, op, fill, comb):
            red = [[op(jnp.where(mk, vals[t], fill), axis=1, keepdims=True) for mk in masks[t]] for t in range(5)]
            for t in range(4):
                both = comb(red[t][-1], red[t + 1][0])
                red[t][-1] = both
                red[t + 1][0] = both
            out = []
            for t in range(5):
                b = red[t][0]
                for n in range(1, len(red[t])):
                    b = jnp.where(lane >= _PARTS[t][n][1], red[t][n], b)
                out.append(b)
            return out
        mx = reduce(sg, jnp.max, -jnp.inf, jnp.maximum)
        e = [jnp.exp(sg[t] - mx[t]) for t in range(5)]
        l = reduce(e, jnp.sum, 0.0, jnp.add)
        ps = []
        for t in range(5):
            r = pl.reciprocal(l[t], approx=True)
            r = r * (2.0 - l[t] * r)
            ps.append(e[t] * r)
        return jnp.concatenate(ps, axis=1)

    def ffn1(r0, slot):
        hid = _dot(xn_scr[pl.ds(r0, SEG), :], _unpack(w1_scr[...]))
        hh = 0.5 * hid
        hid_scr[slot] = _pack(hh * jnp.tanh(hh) + hh)

    ffn1(0, 0)

    def step(r0, rnext, i, m):
        xs = xn_scr[pl.ds(r0, SEG), :]
        h = jnp.concatenate([m, xs], axis=0)
        tall = stacks([proj(h, p) for p in range(8)])
        upr = [proj(h, 8 + p) for p in range(NU0)]
        hr = h[:, 384:512]
        haug = jnp.concatenate([h[:, :384], hr + pltpu.roll(hr, 64, 1)], axis=1)
        if XT:
            tt_scr[...] = pltpu.bitcast(tall.T, u32)
            sc = _dot(haug, _unpack(tt_scr[...]))
        else:
            sc = _dot(haug, tall, NT)
        upr += [proj(h, 8 + p) for p in range(NU0, 8)]
        pfull = softmax(sc)
        uall = stacks(upr)
        ffn1(rnext, (i + 1) % 2)
        oa = _dot(pfull, uall)
        o3 = oa[:, 384:512]
        o = jnp.concatenate([oa[:, :384], jnp.where(low, o3 + pltpu.roll(o3, 64, 1), 0.0)], axis=1)
        ffn = _dot(_unpack(hid_scr[i % 2]), _unpack(w2_scr[...]))
        res_scr[i * SEG:(i + 1) * SEG, :] = o[M:L] + ffn
        return o[0:M].astype(bf16).astype(f32)

    def emit(blk, res):
        c0 = pl.multiple_of(blk * 128, 128)
        rt = res.T[0:D, :]
        out_scr[blk] = (x_scr[:, pl.ds(c0, 128)].astype(f32) + rt).astype(bf16)

    def out_copy(blk):
        c0 = pl.multiple_of(blk * 128, 128)
        return pltpu.make_async_copy(out_scr.at[blk], out_hbm.at[:, pl.ds(c0, 128)], osems.at[blk])

    def body(it, m):
        emit(jnp.maximum(it - 1, 0), res_scr[...])
        for i in range(UNROLL):
            r0 = pl.multiple_of(it * 128 + i * SEG, SEG)
            rnext = pl.multiple_of(jnp.minimum(r0 + SEG, S - SEG), SEG)
            m = step(r0, rnext, i, m)

        @pl.when(it > 0)
        def _():
            out_copy(it - 1).start()
        return m

    m0 = jnp.concatenate([mem_ref[...].astype(f32), jnp.zeros((M, DP - D), f32)], axis=1)
    jax.lax.fori_loop(0, NBLK, body, m0)
    emit(NBLK - 1, res_scr[...])
    out_copy(NBLK - 1).start()
    for b in range(NBLK):
        out_copy(b).wait()


@jax.jit
def run(A_x, A_mem0, A_Wq, A_Wk, A_Wv, A_Wo, B_w1, B_w2):
    vm = pl.BlockSpec(memory_space=pltpu.VMEM)
    anyspec = pl.BlockSpec(memory_space=pl.ANY)
    out_t = pl.pallas_call(
        kernel,
        out_shape=jax.ShapeDtypeStruct((D, S), bf16),
        in_specs=[anyspec, vm, anyspec, anyspec, anyspec, anyspec, anyspec, anyspec],
        out_specs=anyspec,
        scratch_shapes=[
            pltpu.VMEM((2, D * H, 128), bf16),
            pltpu.VMEM((2, D * H, 128), bf16),
            pltpu.VMEM((2, D * H, 128), bf16),
            pltpu.VMEM((H, D, DH), bf16),
            pltpu.VMEM((D, S), bf16),
            pltpu.VMEM((D, F), bf16),
            pltpu.VMEM((D, F), bf16),
            pltpu.SemaphoreType.DMA((10,)),
            pltpu.SemaphoreType.DMA((NBLK,)),
            pltpu.VMEM((16, DP // 2, 896), u32),
            pltpu.VMEM((S, DP), f32),
            pltpu.VMEM((DP // 2, F), u32),
            pltpu.VMEM((F // 2, DP), u32),
            pltpu.VMEM((128, DP), f32),
            pltpu.VMEM((NBLK, D, 128), bf16),
            pltpu.VMEM((2, SEG // 2, F), u32),
            pltpu.VMEM((DP // 2, 640), u32),
        ],
        compiler_params=pltpu.CompilerParams(vmem_limit_bytes=120 * 1024 * 1024),
    )(jnp.swapaxes(A_x, 1, 2).reshape(D, S), A_mem0.reshape(M, D), A_Wq.reshape(D * H, DH),
      A_Wk.reshape(D * H, DH), A_Wv.reshape(D * H, DH), jnp.swapaxes(A_Wo, 1, 2), B_w1, B_w2.T)
    return jnp.swapaxes(out_t.reshape(1, D, S), 1, 2)


def pallas_parallel_sum__memory_aug_recurrent_mem_tr__dense_activation_silu__prompt_kernel(A_x, A_mem0, A_Wq, A_Wk, A_Wv, A_Wo, A_seg_len, B_x, B_w1, B_w2):
    return run(A_x, A_mem0, A_Wq, A_Wk, A_Wv, A_Wo, B_w1, B_w2)
```

```python
import jax
import jax.numpy as jnp
import numpy as np
from jax.experimental import pallas as pl
from jax.experimental.pallas import tpu as pltpu

S, D, H, DH, M, SEG, F = 2048, 448, 16, 256, 8, 32, 1792
NSEG = S // SEG
L = M + SEG
DP = 512
DM = 384
UNROLL = 4
NBLK = S // 128
f32, bf16, u32 = jnp.float32, jnp.bfloat16, jnp.uint32
NT = (((1,), (1,)), ((), ()))
NN = (((1,), (0,)), ((), ()))
NU0 = 2


def _dot(a, b, dims=NN):
    return jax.lax.dot_general(a, b, dims, preferred_element_type=f32)


def _pack(x):
    return pltpu.bitcast(x.astype(bf16), u32)


def _unpack(x):
    return pltpu.bitcast(x, bf16)


_PARTS = [[(j, max(40 * j, 128 * t) - 128 * t, min(40 * j + 40, 128 * t + 128) - 128 * t)
           for j in range(H) if 40 * j < 128 * t + 128 and 40 * j + 40 > 128 * t] for t in range(5)]
TAILV = True
ZT = True
_FV = 3
_FCH = [[(0, 512), (512, 512), (1024, 384), (1408, 384)],
        [(0, 384), (384, 384), (768, 512), (1280, 512)],
        [(0, 512), (512, 384), (896, 512), (1408, 384)],
        [(0, 384), (384, 512), (896, 384), (1280, 512)]][_FV]
_ORD = 1
_FILL = [[(1, 0), (1, 1), (1, 2), (1, 3), (2, 0), (2, 1), (2, 2), (2, 3)],
         [(1, 0), (1, 1), (2, 0), (1, 2), (2, 1), (1, 3), (2, 2), (2, 3)],
         [(1, 0), (1, 1), (1, 2), (2, 0), (1, 3), (2, 1), (2, 2), (2, 3)]][_ORD]


def kernel(x_hbm, mem_ref, wq_hbm, wk_hbm, wv_hbm, wo_hbm, w1_hbm, w2_hbm, out_hbm,
           q_scr, k_scr, v_scr, wo_scr, x_scr, w1_raw, w2_raw, sems, osems,
           w_scr, wq_scr, wb_scr, xn_scr, res_scr, out_scr, hid_scr, bt_scr, tt_scr, zt_scr, qh_scr):
    CH = [(0, 128), (128, 128), (256, 128), (384, 64)]
    nsem = [0]

    def copy(src, dst):
        nsem[0] += 1
        return pltpu.make_async_copy(src, dst, sems.at[nsem[0] - 1])

    def chunk(src, dst, i):
        r0, n = CH[i][0] * H, CH[i][1] * H
        return [copy(src.at[pl.ds(r0, n), pl.ds(c * 128, 128)], dst.at[c, pl.ds(r0, n), :]) for c in range(2)]
    cq = [chunk(wq_hbm, q_scr, i) for i in range(4)]
    ck = [chunk(wk_hbm, k_scr, i) for i in range(4)]
    cv = [chunk(wv_hbm, v_scr, i) for i in range(4)]
    co = [copy(wo_hbm.at[pl.ds(8 * i, 8)], wo_scr.at[pl.ds(8 * i, 8)]) for i in range(2)]
    cx = [copy(x_hbm.at[:, pl.ds(a, b - a)], x_scr.at[:, pl.ds(a, b - a)])
          for a, b in ((0, 128), (128, 896), (896, S))]
    c1 = [copy(w1_hbm.at[:, pl.ds(f0, fn)], w1_raw.at[:, pl.ds(f0, fn)]) for f0, fn in _FCH]
    c2 = copy(w2_hbm, w2_raw)

    def start(*cs):
        for c in cs:
            for d in (c if isinstance(c, list) else [c]):
                d.start()

    def wait(*cs):
        for c in cs:
            for d in (c if isinstance(c, list) else [c]):
                d.wait()

    start(cx[0], cx[1], c1, ck[0], cq[0], cq[1], cq[2], cq[3], ck[1], ck[2], ck[3], cv[0], co[0], co[1],
          cv[1], cv[2], cv[3], c2, cx[2])
    res_scr[...] = jnp.zeros((128, DP), f32)
    bt_scr[...] = jnp.zeros((D, 128), f32)

    def get(scr, p, r0, n, mul=None):
        los, his = [], []
        for c in range(2):
            x = scr.at[c].bitcast(u32)[pl.ds(p + 8 * r0, n, stride=8), :]
            los.append(pltpu.bitcast(x << 16, f32))
            his.append(pltpu.bitcast(x & jnp.uint32(0xffff0000), f32))
        lo, hi = jnp.concatenate(los, axis=1), jnp.concatenate(his, axis=1)
        if mul is not None:
            lo, hi = lo * mul, hi * mul
        return lo, hi

    def put(idx, i, e, o):
        r0, n = CH[i][0] // 2, CH[i][1] // 2
        if i < 3:
            w_scr[idx, r0:r0 + n, :] = jnp.concatenate(
                [_pack(e[:, :384]), _pack(o[:, :384]),
                 _pack(jnp.concatenate([e[:, 384:448], o[:, 384:448]], axis=1))], axis=1)
            return
        t = jnp.concatenate([e, o], axis=0)
        if idx < 8:
            wq_scr[:, idx * 128:(idx + 1) * 128] = _pack(jnp.concatenate([t, t[:, 384:448]], axis=1).T)
        else:
            wb_scr[(idx - 8) * 64:(idx - 7) * 64, :] = _pack(
                jnp.concatenate([t, jnp.zeros((128, DP - D), f32)], axis=1))

    scale = DH ** -0.5

    def chunk_loop(compute, store, nxt, pairs=range(8), extra=None):
        for p in pairs:
            e, o = compute(p)
            if p == pairs[-1] and nxt:
                wait(*nxt)
            store(p, e, o)
            if extra is not None:
                extra(p)

    def m_rows(i, nxt):
        def compute(p):
            klo, khi = get(k_scr, p, CH[i][0], CH[i][1], scale)
            if i == 0:
                qlo, qhi = (t.astype(bf16) for t in get(q_scr, p, 0, D))
                qh_scr[2 * p] = pltpu.bitcast(qlo, u32)
                qh_scr[2 * p + 1] = pltpu.bitcast(qhi, u32)
            else:
                qlo, qhi = _unpack(qh_scr[2 * p]), _unpack(qh_scr[2 * p + 1])
            return _dot(klo, qlo, NT), _dot(khi, qhi, NT)
        chunk_loop(compute, lambda p, e, o: put(p, i, e, o), nxt)

    def b_rows(i, nxt, pairs=range(8), extra=None):
        def compute(p):
            vlo, vhi = get(v_scr, p, CH[i][0], CH[i][1])
            return _dot(vlo, wo_scr[2 * p], NT), _dot(vhi, wo_scr[2 * p + 1], NT)
        chunk_loop(compute, lambda p, e, o: put(p + 8, i, e, o), nxt, pairs, extra)

    def layernorm(c0):
        xb = x_scr[:, pl.ds(c0, 128)].astype(f32)
        mu = jnp.mean(xb, axis=0, keepdims=True)
        xc = xb - mu
        var = jnp.mean(xc * xc, axis=0, keepdims=True)
        xn = (xc * jax.lax.rsqrt(var + 1e-5)).astype(bf16).astype(f32)
        xn = jnp.concatenate([xn, jnp.zeros((DP - D, 128), f32)], axis=0)
        xn_scr[pl.ds(c0, 128), :] = xn.T

    def ffn1(r0, h0, rows, n):
        f0, fn = _FCH[n]
        hid = _dot(xn_scr[pl.ds(r0, rows), 0:D], w1_raw[:, f0:f0 + fn])
        hh = 0.5 * hid
        hid_scr[pl.ds(h0, rows // 2), f0:f0 + fn] = _pack(hh * jnp.tanh(hh) + hh)

    wait(cx[0])
    layernorm(0)
    wait(cx[1], c1[0])
    for b in range(6):
        layernorm(128 * (b + 1))
        ffn1(128 * b, 64 * b, 128, 0)
    wait(c1[1], c1[2], c1[3])
    for n in range(1, 4):
        for b in range(6):
            ffn1(128 * b, 64 * b, 128, n)
    wait(ck[0], cq[0], cq[1], cq[2], cq[3])
    m_rows(0, [ck[1], ck[2], ck[3]])
    m_rows(1, None)
    m_rows(2, None)
    m_rows(3, [cv[0], co[0], co[1]])
    b_rows(0, [cv[1], cv[2], cv[3]])
    b_rows(1, None)
    b_rows(2, None)
    b_rows(3, [c2, cx[2]])

    lane = jax.lax.broadcasted_iota(jnp.int32, (L, 128), 1)
    row = jax.lax.broadcasted_iota(jnp.int32, (L, 128), 0)
    low = lane < 64

    def proj(h, idx):
        return _dot(h[:, 0:DM], _unpack(w_scr[idx]))

    def key_blocks(haug):
        rem = haug[:, 384:512]
        par = [jnp.where(low, rem, 0.0), jnp.where(low, 0.0, rem)]
        z = {}
        for t in range(5):
            for j in sorted({hd // 2 for hd, _, _ in _PARTS[t]}):
                rows = []
                for hd, lo, hi in _PARTS[t]:
                    k0 = 128 * t + lo - 40 * hd
                    rows.append(par[hd % 2][k0:k0 + hi - lo] if hd // 2 == j
                                else jnp.zeros((hi - lo, 128), f32))
                z[t, j] = jnp.concatenate(rows, axis=0).astype(bf16)
        return z

    def stacks(pr):
        rows = []
        for r in pr:
            rem = r[:, 768:896]
            rows.append(jnp.concatenate([r[:, 0:384], jnp.where(low, rem, 0.0)], axis=1))
            rows.append(jnp.concatenate([r[:, 384:768], jnp.where(low, 0.0, rem)], axis=1))
        return jnp.concatenate(rows, axis=0).astype(bf16)

    def softmax(sc):
        sg, masks = [], []
        for t in range(5):
            col = lane + 128 * t
            key = col
            for (j, lo, hi) in _PARTS[t]:
                key = jnp.where(lane >= lo, col - 40 * j, key)
            valid = (row < M) | (row >= key)
            sg.append(jnp.where(valid, sc[:, t * 128:(t + 1) * 128], -1e9))
            masks.append([(lane >= lo) & (lane < hi) for (_, lo, hi) in _PARTS[t]])

        def reduce(vals, op, fill, comb):
            red = [[op(jnp.where(mk, vals[t], fill), axis=1, keepdims=True) for mk in masks[t]] for t in range(5)]
            for t in range(4):
                both = comb(red[t][-1], red[t + 1][0])
                red[t][-1] = both
                red[t + 1][0] = both
            out = []
            for t in range(5):
                b = red[t][0]
                for n in range(1, len(red[t])):
                    b = jnp.where(lane >= _PARTS[t][n][1], red[t][n], b)
                out.append(b)
            return out
        mx = reduce(sg, jnp.max, -jnp.inf, jnp.maximum)
        e = [jnp.exp(sg[t] - mx[t]) for t in range(5)]
        l = reduce(e, jnp.sum, 0.0, jnp.add)
        ps = []
        for t in range(5):
            r = pl.reciprocal(l[t], approx=True)
            r = r * (2.0 - l[t] * r)
            ps.append(e[t] * r)
        return jnp.concatenate(ps, axis=1)

    def ffn2(blk, n):
        f0, fn = _FCH[n]
        hid = _unpack(hid_scr[pl.ds(pl.multiple_of(blk * 64, 64), 64), f0:f0 + fn])
        part = _dot(w2_raw[:, f0:f0 + fn], hid, NT)
        if n == 0:
            bt_scr[...] = part
        else:
            bt_scr[...] += part

    def filler(blk, g):
        stage, n = _FILL[g]
        if stage == 1:
            ffn1(pl.multiple_of(768 + 80 * blk, 8), pl.multiple_of(384 + 40 * blk, 8), 80, n)
        else:
            ffn2(blk, n)

    def step(blk, i, m):
        c0 = blk * 128
        xs = xn_scr[pl.ds(pl.multiple_of(c0 + i * SEG, SEG), SEG), :]
        h = jnp.concatenate([m, xs], axis=0)
        hr = h[:, 384:512]
        haug = jnp.concatenate([h[:, :384], hr + pltpu.roll(hr, 64, 1)], axis=1)
        z = key_blocks(haug)
        tall = stacks([proj(h, p) for p in range(8)])
        qr = _dot(h, _unpack(wq_scr[...]))
        upr = [proj(h, 8 + p) for p in range(NU0)]
        tt_scr[...] = pltpu.bitcast(tall.T, u32)
        sc = _dot(haug, _unpack(tt_scr[...]))
        if ZT:
            for n, key in enumerate(z):
                zt_scr[n] = pltpu.bitcast(z[key].T, u32)
            zt = {key: _unpack(zt_scr[n]) for n, key in enumerate(z)}
            sc = sc + jnp.concatenate(
                [sum(_dot(qr[:, j * 128:(j + 1) * 128], zt[t, j]) for (tt, j) in z if tt == t)
                 for t in range(5)], axis=1)
        else:
            sc = sc + jnp.concatenate(
                [sum(_dot(qr[:, j * 128:(j + 1) * 128], z[t, j], NT) for (tt, j) in z if tt == t)
                 for t in range(5)], axis=1)
        upr += [proj(h, 8 + p) for p in range(NU0, 8)]
        pfull = softmax(sc)
        uall = stacks(upr)
        yr = jnp.concatenate(
            [sum(_dot(pfull[:, t * 128:(t + 1) * 128], z[t, j]) for (t, jj) in z if jj == j)
             for j in range(8)], axis=1)
        filler(blk, 2 * i)
        last = i == UNROLL - 1 and TAILV
        o = _dot(pfull, uall)
        if last:
            filler(blk, 2 * i + 1)
        o = o + _dot(yr, _unpack(wb_scr[...]))
        if not last:
            filler(blk, 2 * i + 1)
        res_scr[i * SEG:(i + 1) * SEG, :] = o[M:L]
        return o[0:M]

    def emit(blk):
        c0 = pl.multiple_of(blk * 128, 128)
        rt = res_scr[...].T
        rt = jnp.concatenate([rt[0:384], rt[384:448] + rt[448:512]], axis=0)
        out_scr[blk] = (x_scr[:, pl.ds(c0, 128)].astype(f32) + rt + bt_scr[...]).astype(bf16)

    def out_dma(blk):
        c0 = pl.multiple_of(blk * 128, 128)
        return pltpu.make_async_copy(out_scr.at[blk], out_hbm.at[:, pl.ds(c0, 128)], osems.at[blk])

    def body(blk, m):
        emit(jnp.maximum(blk - 1, 0))
        for i in range(UNROLL):
            m = step(blk, i, m)
        layernorm(pl.multiple_of(jnp.minimum(blk + 7, NBLK - 1) * 128, 128))

        @pl.when(blk > 0)
        def _():
            out_dma(blk - 1).start()
        return m

    m0 = jnp.concatenate([mem_ref[...].astype(f32), jnp.zeros((M, DP - D), f32)], axis=1)
    jax.lax.fori_loop(0, NBLK, body, m0)
    emit(NBLK - 1)
    out_dma(NBLK - 1).start()
    for b in range(NBLK):
        out_dma(b).wait()


@jax.jit
def run(A_x, A_mem0, A_Wq, A_Wk, A_Wv, A_Wo, B_w1, B_w2):
    vm = pl.BlockSpec(memory_space=pltpu.VMEM)
    anyspec = pl.BlockSpec(memory_space=pl.ANY)
    out_t = pl.pallas_call(
        kernel,
        out_shape=jax.ShapeDtypeStruct((D, S), bf16),
        in_specs=[anyspec, vm, anyspec, anyspec, anyspec, anyspec, anyspec, anyspec],
        out_specs=anyspec,
        scratch_shapes=[
            pltpu.VMEM((2, D * H, 128), bf16),
            pltpu.VMEM((2, D * H, 128), bf16),
            pltpu.VMEM((2, D * H, 128), bf16),
            pltpu.VMEM((H, D, DH), bf16),
            pltpu.VMEM((D, S), bf16),
            pltpu.VMEM((D, F), bf16),
            pltpu.VMEM((D, F), bf16),
            pltpu.SemaphoreType.DMA((32,)),
            pltpu.SemaphoreType.DMA((NBLK,)),
            pltpu.VMEM((16, DM // 2, 896), u32),
            pltpu.VMEM((DP // 2, 1024), u32),
            pltpu.VMEM((512, DP), u32),
            pltpu.VMEM((S, DP), f32),
            pltpu.VMEM((128, DP), f32),
            pltpu.VMEM((NBLK, D, 128), bf16),
            pltpu.VMEM((S // 2, F), u32),
            pltpu.VMEM((D, 128), f32),
            pltpu.VMEM((DP // 2, 640), u32),
            pltpu.VMEM((12, 64, 128), u32),
            pltpu.VMEM((H, D // 2, DH), u32),
        ],
        compiler_params=pltpu.CompilerParams(vmem_limit_bytes=120 * 1024 * 1024),
    )(jnp.swapaxes(A_x, 1, 2).reshape(D, S), A_mem0.reshape(M, D), A_Wq.reshape(D * H, DH),
      A_Wk.reshape(D * H, DH), A_Wv.reshape(D * H, DH), jnp.swapaxes(A_Wo, 1, 2), B_w1, B_w2.T)
    return jnp.swapaxes(out_t.reshape(1, D, S), 1, 2)


def pallas_parallel_sum__memory_aug_recurrent_mem_tr__dense_activation_silu__prompt_kernel(A_x, A_mem0, A_Wq, A_Wk, A_Wv, A_Wo, A_seg_len, B_x, B_w1, B_w2):
    return run(A_x, A_mem0, A_Wq, A_Wk, A_Wv, A_Wo, B_w1, B_w2)
```

```python
import jax
import jax.numpy as jnp
import numpy as np
from jax.experimental import pallas as pl
from jax.experimental.pallas import tpu as pltpu

S, D, H, DH, M, SEG, F = 2048, 448, 16, 256, 8, 32, 1792
NSEG = S // SEG
L = M + SEG
DP = 512
DM = 384
UNROLL = 4
NBLK = S // 128
f32, bf16, u32 = jnp.float32, jnp.bfloat16, jnp.uint32
NT = (((1,), (1,)), ((), ()))
NN = (((1,), (0,)), ((), ()))
NU0 = 3


def _dot(a, b, dims=NN):
    return jax.lax.dot_general(a, b, dims, preferred_element_type=f32)


def _pack(x):
    return pltpu.bitcast(x.astype(bf16), u32)


def _unpack(x):
    return pltpu.bitcast(x, bf16)


_PARTS = [[(j, max(40 * j, 128 * t) - 128 * t, min(40 * j + 40, 128 * t + 128) - 128 * t)
           for j in range(H) if 40 * j < 128 * t + 128 and 40 * j + 40 > 128 * t] for t in range(5)]
TAILV = True
_GROUPS = [[tuple(sorted((p[i][0], p[i + 1][0]), key=lambda hd: hd % 2)) for i in (0, 2)] for p in _PARTS]
NSEM = 34
_FV = 3
_FCH = [[(0, 512), (512, 512), (1024, 384), (1408, 384)],
        [(0, 384), (384, 384), (768, 512), (1280, 512)],
        [(0, 512), (512, 384), (896, 512), (1408, 384)],
        [(0, 384), (384, 512), (896, 384), (1280, 512)]][_FV]
_ORD = 2
_FILL = [[(1, 0), (1, 1), (1, 2), (1, 3), (2, 0), (2, 1), (2, 2), (2, 3)],
         [(1, 0), (1, 1), (2, 0), (1, 2), (2, 1), (1, 3), (2, 2), (2, 3)],
         [(1, 0), (1, 1), (1, 2), (2, 0), (1, 3), (2, 1), (2, 2), (2, 3)]][_ORD]


def kernel(x_hbm, mem_ref, wq_hbm, wk_hbm, wv_hbm, wo_hbm, w1_hbm, w2_hbm, out_hbm,
           q_scr, k_scr, v_scr, wo_scr, x_scr, w1_raw, w2_raw, sems, osems,
           w_scr, wq_scr, wb_scr, xn_scr, res_scr, out_scr, hid_scr, bt_scr, tt_scr, zt_scr, qh_scr):
    CH = [(0, 128), (128, 128), (256, 128), (384, 64)]
    nsem = [0]

    def copy(src, dst):
        nsem[0] += 1
        return pltpu.make_async_copy(src, dst, sems.at[nsem[0] - 1])

    def chunk(src, dst, i):
        r0, n = CH[i][0] * H, CH[i][1] * H
        return [copy(src.at[pl.ds(r0, n), pl.ds(c * 128, 128)], dst.at[c, pl.ds(r0, n), :]) for c in range(2)]
    cq = [chunk(wq_hbm, q_scr, i) for i in range(4)]
    ck = [chunk(wk_hbm, k_scr, i) for i in range(4)]
    cv = [chunk(wv_hbm, v_scr, i) for i in range(4)]
    co = [copy(wo_hbm.at[pl.ds(8 * i, 8)], wo_scr.at[pl.ds(8 * i, 8)]) for i in range(2)]
    cx = [copy(x_hbm.at[:, pl.ds(a, b - a)], x_scr.at[:, pl.ds(a, b - a)])
          for a, b in ((0, 128), (128, 896), (896, S))]
    c1 = [copy(w1_hbm.at[:, pl.ds(f0, fn)], w1_raw.at[:, pl.ds(f0, fn)]) for f0, fn in _FCH]
    c2 = copy(w2_hbm, w2_raw)

    assert nsem[0] == NSEM

    def start(*cs):
        for c in cs:
            for d in (c if isinstance(c, list) else [c]):
                d.start()

    def wait(*cs):
        for c in cs:
            for d in (c if isinstance(c, list) else [c]):
                d.wait()

    start(cx[0], cx[1], c1, ck[0], cq[0], cq[1], cq[2], cq[3], ck[1], ck[2], ck[3], cv[0], co[0], co[1],
          cv[1], cv[2], cv[3], c2, cx[2])
    res_scr[...] = jnp.zeros((128, DP), f32)
    bt_scr[...] = jnp.zeros((D, 128), f32)

    def get(scr, p, r0, n, mul=None):
        los, his = [], []
        for c in range(2):
            x = scr.at[c].bitcast(u32)[pl.ds(p + 8 * r0, n, stride=8), :]
            los.append(pltpu.bitcast(x << 16, f32))
            his.append(pltpu.bitcast(x & jnp.uint32(0xffff0000), f32))
        lo, hi = jnp.concatenate(los, axis=1), jnp.concatenate(his, axis=1)
        if mul is not None:
            lo, hi = lo * mul, hi * mul
        return lo, hi

    def put(idx, i, e, o):
        if i < 3:
            w_scr[idx, 64 * i:64 * (i + 1), 0:768] = jnp.concatenate([_pack(e), _pack(o)], axis=1)
            return
        w_scr[idx, :, 768:896] = _pack(jnp.concatenate([e[1], o[1]], axis=0).T)
        t = jnp.concatenate([e[0], o[0]], axis=0)
        if idx < 8:
            wq_scr[:, idx * 128:(idx + 1) * 128] = _pack(jnp.concatenate([t, t[:, 384:448]], axis=1).T)
        else:
            wb_scr[(idx - 8) * 64:(idx - 7) * 64, :] = _pack(
                jnp.concatenate([t, jnp.zeros((128, DP - D), f32)], axis=1))

    scale = DH ** -0.5

    def chunk_loop(compute, store, nxt, pairs=range(8), extra=None):
        for p in pairs:
            e, o = compute(p)
            if p == pairs[-1] and nxt:
                wait(*nxt)
            store(p, e, o)
            if extra is not None:
                extra(p)

    def product(i, lhs, rhs):
        def one(par):
            if i < 3:
                return _dot(lhs(128 * i, 128)[par], rhs[par][0:DM], NT)
            return (_dot(lhs(DM, 64)[par], rhs[par], NT),
                    _dot(rhs[par][DM:D], lhs(0, DM)[par].astype(bf16), NT))
        return one(0), one(1)

    def m_rows(i, nxt):
        def compute(p):
            if i == 0:
                q = [t.astype(bf16) for t in get(q_scr, p, 0, DM)]
                qh_scr[2 * p] = pltpu.bitcast(q[0], u32)
                qh_scr[2 * p + 1] = pltpu.bitcast(q[1], u32)
            else:
                q = [_unpack(qh_scr[2 * p]), _unpack(qh_scr[2 * p + 1])]
            if i == 3:
                q = [jnp.concatenate([a, b.astype(bf16)], axis=0) for a, b in zip(q, get(q_scr, p, DM, 64))]
            return product(i, lambda r0, n: get(k_scr, p, r0, n, scale), q)
        chunk_loop(compute, lambda p, e, o: put(p, i, e, o), nxt)

    def b_rows(i, nxt):
        def compute(p):
            return product(i, lambda r0, n: get(v_scr, p, r0, n), [wo_scr[2 * p], wo_scr[2 * p + 1]])
        chunk_loop(compute, lambda p, e, o: put(p + 8, i, e, o), nxt)

    def layernorm(c0):
        xb = x_scr[:, pl.ds(c0, 128)].astype(f32)
        mu = jnp.mean(xb, axis=0, keepdims=True)
        xc = xb - mu
        var = jnp.mean(xc * xc, axis=0, keepdims=True)
        xn = (xc * jax.lax.rsqrt(var + 1e-5)).astype(bf16).astype(f32)
        xn = jnp.concatenate([xn, jnp.zeros((DP - D, 128), f32)], axis=0)
        xn_scr[pl.ds(c0, 128), :] = xn.T

    def ffn1(r0, h0, rows, n):
        f0, fn = _FCH[n]
        hid = _dot(xn_scr[pl.ds(r0, rows), 0:D], w1_raw[:, f0:f0 + fn])
        hh = 0.5 * hid
        hid_scr[pl.ds(h0, rows // 2), f0:f0 + fn] = _pack(hh * jnp.tanh(hh) + hh)

    wait(cx[0])
    layernorm(0)
    wait(cx[1], c1[0])
    for b in range(6):
        layernorm(128 * (b + 1))
        ffn1(128 * b, 64 * b, 128, 0)
    wait(c1[1], c1[2], c1[3])
    for n in range(1, 4):
        for b in range(6):
            ffn1(128 * b, 64 * b, 128, n)
    wait(ck[0], cq[0], cq[1], cq[2])
    m_rows(0, [cq[3], ck[1], ck[2], ck[3]])
    m_rows(1, None)
    m_rows(2, None)
    m_rows(3, [cv[0], co[0], co[1]])
    b_rows(0, [cv[1], cv[2], cv[3]])
    b_rows(1, None)
    b_rows(2, None)
    b_rows(3, [c2, cx[2]])

    lane = jax.lax.broadcasted_iota(jnp.int32, (L, 128), 1)
    row = jax.lax.broadcasted_iota(jnp.int32, (L, 128), 0)
    low = lane < 64

    def proj(h, idx):
        return _dot(h[:, 0:DM], _unpack(w_scr[idx]))

    def key_blocks(haug):
        rem = haug[:, 384:512]
        par = [jnp.where(low, rem, 0.0), jnp.where(low, 0.0, rem)]
        z = {}
        for t in range(5):
            for g in _GROUPS[t]:
                rows = []
                for hd, lo, hi in _PARTS[t]:
                    k0 = 128 * t + lo - 40 * hd
                    rows.append(par[hd % 2][k0:k0 + hi - lo] if hd in g else jnp.zeros((hi - lo, 128), f32))
                z[t, g] = jnp.concatenate(rows, axis=0).astype(bf16)
        return z

    def stacks(pr):
        rows = []
        for r in pr:
            rem = r[:, 768:896]
            rows.append(jnp.concatenate([r[:, 0:384], jnp.where(low, rem, 0.0)], axis=1))
            rows.append(jnp.concatenate([r[:, 384:768], jnp.where(low, 0.0, rem)], axis=1))
        return jnp.concatenate(rows, axis=0).astype(bf16)

    def softmax(sc):
        sg, masks = [], []
        for t in range(5):
            col = lane + 128 * t
            key = col
            for (j, lo, hi) in _PARTS[t]:
                key = jnp.where(lane >= lo, col - 40 * j, key)
            valid = (row < M) | (row >= key)
            sg.append(jnp.where(valid, sc[:, t * 128:(t + 1) * 128], -1e9))
            masks.append([(lane >= lo) & (lane < hi) for (_, lo, hi) in _PARTS[t]])

        def reduce(vals, op, fill, comb):
            red = [[op(jnp.where(mk, vals[t], fill), axis=1, keepdims=True) for mk in masks[t]] for t in range(5)]
            for t in range(4):
                both = comb(red[t][-1], red[t + 1][0])
                red[t][-1] = both
                red[t + 1][0] = both
            out = []
            for t in range(5):
                b = red[t][0]
                for n in range(1, len(red[t])):
                    b = jnp.where(lane >= _PARTS[t][n][1], red[t][n], b)
                out.append(b)
            return out
        mx = reduce(sg, jnp.max, -jnp.inf, jnp.maximum)
        e = [jnp.exp(sg[t] - mx[t]) for t in range(5)]
        l = reduce(e, jnp.sum, 0.0, jnp.add)
        ps = []
        for t in range(5):
            r = pl.reciprocal(l[t], approx=True)
            r = r * (2.0 - l[t] * r)
            ps.append(e[t] * r)
        return jnp.concatenate(ps, axis=1)

    def ffn2(blk, n):
        f0, fn = _FCH[n]
        hid = _unpack(hid_scr[pl.ds(pl.multiple_of(blk * 64, 64), 64), f0:f0 + fn])
        part = _dot(w2_raw[:, f0:f0 + fn], hid, NT)
        if n == 0:
            bt_scr[...] = part
        else:
            bt_scr[...] += part

    def filler(blk, g):
        stage, n = _FILL[g]
        if stage == 1:
            ffn1(pl.multiple_of(768 + 80 * blk, 8), pl.multiple_of(384 + 40 * blk, 8), 80, n)
        else:
            ffn2(blk, n)

    def step(blk, i, m):
        c0 = blk * 128
        xs = xn_scr[pl.ds(pl.multiple_of(c0 + i * SEG, SEG), SEG), :]
        h = jnp.concatenate([m, xs], axis=0)
        hr = h[:, 384:512]
        haug = jnp.concatenate([h[:, :384], hr + pltpu.roll(hr, 64, 1)], axis=1)
        z = key_blocks(haug)
        tall = stacks([proj(h, p) for p in range(8)])
        qr = _dot(h, _unpack(wq_scr[...]))
        upr = [proj(h, 8 + p) for p in range(NU0)]
        tt_scr[...] = pltpu.bitcast(tall.T, u32)
        sc = _dot(haug, _unpack(tt_scr[...]))
        for n, key in enumerate(z):
            zt_scr[n] = pltpu.bitcast(z[key].T, u32)

        def qpair(g):
            he, ho = qr[:, (g[0] // 2) * 128:(g[0] // 2 + 1) * 128], qr[:, (g[1] // 2) * 128:(g[1] // 2 + 1) * 128]
            return he if g[0] // 2 == g[1] // 2 else jnp.where(low, he, ho)
        zt = {key: _unpack(zt_scr[n]) for n, key in enumerate(z)}
        sc = sc + jnp.concatenate(
            [sum(_dot(qpair(g), zt[t, g]) for g in _GROUPS[t]) for t in range(5)], axis=1)
        upr += [proj(h, 8 + p) for p in range(NU0, 8)]
        pfull = softmax(sc)
        uall = stacks(upr)
        yp = {key: _dot(pfull[:, key[0] * 128:(key[0] + 1) * 128], z[key]) for key in z}
        yr = []
        for j in range(8):
            lo_keys = [k for k in z if k[1][0] == 2 * j]
            hi_keys = [k for k in z if k[1][1] == 2 * j + 1]
            lo_sum = sum(yp[k] for k in lo_keys)
            yr.append(lo_sum if lo_keys == hi_keys else jnp.where(low, lo_sum, sum(yp[k] for k in hi_keys)))
        yr = jnp.concatenate(yr, axis=1)
        filler(blk, 2 * i)
        last = i == UNROLL - 1 and TAILV
        o = _dot(pfull, uall)
        if last:
            filler(blk, 2 * i + 1)
        o = o + _dot(yr, _unpack(wb_scr[...]))
        if not last:
            filler(blk, 2 * i + 1)
        res_scr[i * SEG:(i + 1) * SEG, :] = o[M:L]
        return o[0:M]

    def emit(blk):
        c0 = pl.multiple_of(blk * 128, 128)
        rt = res_scr[...].T
        rt = jnp.concatenate([rt[0:384], rt[384:448] + rt[448:512]], axis=0)
        out_scr[blk] = (x_scr[:, pl.ds(c0, 128)].astype(f32) + rt + bt_scr[...]).astype(bf16)

    def out_dma(blk):
        c0 = pl.multiple_of(blk * 128, 128)
        return pltpu.make_async_copy(out_scr.at[blk], out_hbm.at[:, pl.ds(c0, 128)], osems.at[blk])

    def body(blk, m):
        emit(jnp.maximum(blk - 1, 0))
        for i in range(UNROLL):
            m = step(blk, i, m)
        layernorm(pl.multiple_of(jnp.minimum(blk + 7, NBLK - 1) * 128, 128))

        @pl.when(blk > 0)
        def _():
            out_dma(blk - 1).start()
        return m

    m0 = jnp.concatenate([mem_ref[...].astype(f32), jnp.zeros((M, DP - D), f32)], axis=1)
    jax.lax.fori_loop(0, NBLK, body, m0)
    emit(NBLK - 1)
    out_dma(NBLK - 1).start()
    for b in range(NBLK):
        out_dma(b).wait()


@jax.jit
def run(A_x, A_mem0, A_Wq, A_Wk, A_Wv, A_Wo, B_w1, B_w2):
    vm = pl.BlockSpec(memory_space=pltpu.VMEM)
    anyspec = pl.BlockSpec(memory_space=pl.ANY)
    out_t = pl.pallas_call(
        kernel,
        out_shape=jax.ShapeDtypeStruct((D, S), bf16),
        in_specs=[anyspec, vm, anyspec, anyspec, anyspec, anyspec, anyspec, anyspec],
        out_specs=anyspec,
        scratch_shapes=[
            pltpu.VMEM((2, D * H, 128), bf16),
            pltpu.VMEM((2, D * H, 128), bf16),
            pltpu.VMEM((2, D * H, 128), bf16),
            pltpu.VMEM((H, D, DH), bf16),
            pltpu.VMEM((D, S), bf16),
            pltpu.VMEM((D, F), bf16),
            pltpu.VMEM((D, F), bf16),
            pltpu.SemaphoreType.DMA((NSEM,)),
            pltpu.SemaphoreType.DMA((NBLK,)),
            pltpu.VMEM((16, DM // 2, 896), u32),
            pltpu.VMEM((DP // 2, 1024), u32),
            pltpu.VMEM((512, DP), u32),
            pltpu.VMEM((S, DP), f32),
            pltpu.VMEM((128, DP), f32),
            pltpu.VMEM((NBLK, D, 128), bf16),
            pltpu.VMEM((S // 2, F), u32),
            pltpu.VMEM((D, 128), f32),
            pltpu.VMEM((DP // 2, 640), u32),
            pltpu.VMEM((10, 64, 128), u32),
            pltpu.VMEM((H, DM // 2, DH), u32),
        ],
        compiler_params=pltpu.CompilerParams(vmem_limit_bytes=120 * 1024 * 1024),
    )(jnp.swapaxes(A_x, 1, 2).reshape(D, S), A_mem0.reshape(M, D), A_Wq.reshape(D * H, DH),
      A_Wk.reshape(D * H, DH), A_Wv.reshape(D * H, DH), jnp.swapaxes(A_Wo, 1, 2), B_w1, B_w2.T)
    return jnp.swapaxes(out_t.reshape(1, D, S), 1, 2)


def pallas_parallel_sum__memory_aug_recurrent_mem_tr__dense_activation_silu__prompt_kernel(A_x, A_mem0, A_Wq, A_Wk, A_Wv, A_Wo, A_seg_len, B_x, B_w1, B_w2):
    return run(A_x, A_mem0, A_Wq, A_Wk, A_Wv, A_Wo, B_w1, B_w2)
```

```python
import jax
import jax.numpy as jnp
import numpy as np
from jax.experimental import pallas as pl
from jax.experimental.pallas import tpu as pltpu

S, D, H, DH, M, SEG, F = 2048, 448, 16, 256, 8, 32, 1792
NSEG = S // SEG
L = M + SEG
DP = 512
DM = 384
UNROLL = 4
NBLK = S // 128
f32, bf16, u32 = jnp.float32, jnp.bfloat16, jnp.uint32
NT = (((1,), (1,)), ((), ()))
NN = (((1,), (0,)), ((), ()))
NU0 = 3


def _dot(a, b, dims=NN):
    return jax.lax.dot_general(a, b, dims, preferred_element_type=f32)


def _pack(x):
    return pltpu.bitcast(x.astype(bf16), u32)


def _unpack(x):
    return pltpu.bitcast(x, bf16)


_PARTS = [[(j, max(40 * j, 128 * t) - 128 * t, min(40 * j + 40, 128 * t + 128) - 128 * t)
           for j in range(H) if 40 * j < 128 * t + 128 and 40 * j + 40 > 128 * t] for t in range(5)]
TAILV = True
_GROUPS = [[tuple(sorted((p[i][0], p[i + 1][0]), key=lambda hd: hd % 2)) for i in (0, 2)] for p in _PARTS]
NSEM = 34
_FV = 3
_FCH = [[(0, 512), (512, 512), (1024, 384), (1408, 384)],
        [(0, 384), (384, 384), (768, 512), (1280, 512)],
        [(0, 512), (512, 384), (896, 512), (1408, 384)],
        [(0, 384), (384, 512), (896, 384), (1280, 512)]][_FV]
_ORD = 2
_FILL = [[(1, 0), (1, 1), (1, 2), (1, 3), (2, 0), (2, 1), (2, 2), (2, 3)],
         [(1, 0), (1, 1), (2, 0), (1, 2), (2, 1), (1, 3), (2, 2), (2, 3)],
         [(1, 0), (1, 1), (1, 2), (2, 0), (1, 3), (2, 1), (2, 2), (2, 3)]][_ORD]


def kernel(x_hbm, mem_ref, wq_hbm, wk_hbm, wv_hbm, wo_hbm, w1_hbm, w2_hbm, out_hbm,
           q_scr, k_scr, v_scr, wo_scr, x_scr, w1_raw, w2_raw, sems, osems,
           w_scr, wq_scr, wb_scr, xn_scr, res_scr, out_scr, hid_scr, bt_scr, tt_scr, zt_scr, qh_scr, kh_scr):
    CH = [(0, 128), (128, 128), (256, 128), (384, 64)]
    nsem = [0]

    def copy(src, dst):
        nsem[0] += 1
        return pltpu.make_async_copy(src, dst, sems.at[nsem[0] - 1])

    def chunk(src, dst, i):
        r0, n = CH[i][0] * H, CH[i][1] * H
        return [copy(src.at[pl.ds(r0, n), pl.ds(c * 128, 128)], dst.at[c, pl.ds(r0, n), :]) for c in range(2)]
    cq = [chunk(wq_hbm, q_scr, i) for i in range(4)]
    ck = [chunk(wk_hbm, k_scr, i) for i in range(4)]
    cv = [chunk(wv_hbm, v_scr, i) for i in range(4)]
    co = [copy(wo_hbm.at[:, pl.ds(r0, n), :], wo_scr.at[:, pl.ds(r0, n), :]) for r0, n in ((0, DM), (DM, D - DM))]
    cx = [copy(x_hbm.at[:, pl.ds(a, b - a)], x_scr.at[:, pl.ds(a, b - a)])
          for a, b in ((0, 128), (128, 896), (896, S))]
    c1 = [copy(w1_hbm.at[:, pl.ds(f0, fn)], w1_raw.at[:, pl.ds(f0, fn)]) for f0, fn in _FCH]
    c2 = copy(w2_hbm, w2_raw)

    assert nsem[0] == NSEM

    def start(*cs):
        for c in cs:
            for d in (c if isinstance(c, list) else [c]):
                d.start()

    def wait(*cs):
        for c in cs:
            for d in (c if isinstance(c, list) else [c]):
                d.wait()

    start(cx[0], cx[1], c1, ck[0], cq[0], cq[1], cq[2], ck[1], ck[2], cq[3], ck[3], cv[0], co[0],
          cv[1], cv[2], cv[3], co[1], c2, cx[2])
    res_scr[...] = jnp.zeros((128, DP), f32)
    bt_scr[...] = jnp.zeros((D, 128), f32)

    def get(scr, p, r0, n, mul=None):
        los, his = [], []
        for c in range(2):
            x = scr.at[c].bitcast(u32)[pl.ds(p + 8 * r0, n, stride=8), :]
            los.append(pltpu.bitcast(x << 16, f32))
            his.append(pltpu.bitcast(x & jnp.uint32(0xffff0000), f32))
        lo, hi = jnp.concatenate(los, axis=1), jnp.concatenate(his, axis=1)
        if mul is not None:
            lo, hi = lo * mul, hi * mul
        return lo, hi

    def put(idx, i, e, o):
        if i < 3:
            w_scr[idx, 64 * i:64 * (i + 1), 0:768] = jnp.concatenate([_pack(e), _pack(o)], axis=1)
            return
        w_scr[idx, :, 768:896] = _pack(jnp.concatenate([e[1], o[1]], axis=0).T)
        t = jnp.concatenate([e[0], o[0]], axis=0)
        if idx < 8:
            wq_scr[:, idx * 128:(idx + 1) * 128] = _pack(jnp.concatenate([t, t[:, 384:448]], axis=1).T)
        else:
            wb_scr[(idx - 8) * 64:(idx - 7) * 64, :] = _pack(
                jnp.concatenate([t, jnp.zeros((128, DP - D), f32)], axis=1))

    scale = DH ** -0.5

    def chunk_loop(compute, store, nxt, pairs=range(8), extra=None):
        for p in pairs:
            e, o = compute(p)
            if p == pairs[-1] and nxt:
                wait(*nxt)
            store(p, e, o)
            if extra is not None:
                extra(p)

    def product(i, p, lhs, rhs):
        def one(par, rows):
            if i < 3:
                kh_scr[2 * p + par, 64 * i:64 * (i + 1), :] = _pack(rows[par])
                return _dot(rows[par], rhs[par][0:DM], NT)
            return (_dot(rows[par], rhs[par], NT),
                    _dot(rhs[par][DM:D], _unpack(kh_scr[2 * p + par]), NT))
        rows = lhs(128 * i, 128 if i < 3 else 64)
        return one(0, rows), one(1, rows)

    def m_rows(i, nxt):
        def compute(p):
            if i == 0:
                q = [t.astype(bf16) for t in get(q_scr, p, 0, DM)]
                qh_scr[2 * p] = pltpu.bitcast(q[0], u32)
                qh_scr[2 * p + 1] = pltpu.bitcast(q[1], u32)
            else:
                q = [_unpack(qh_scr[2 * p]), _unpack(qh_scr[2 * p + 1])]
            if i == 3:
                q = [jnp.concatenate([a, b.astype(bf16)], axis=0) for a, b in zip(q, get(q_scr, p, DM, 64))]
            return product(i, p, lambda r0, n: get(k_scr, p, r0, n, scale), q)
        chunk_loop(compute, lambda p, e, o: put(p, i, e, o), nxt)

    def b_rows(i, nxt):
        def compute(p):
            rows = D if i == 3 else DM
            return product(i, p, lambda r0, n: get(v_scr, p, r0, n), [wo_scr[2 * p, 0:rows], wo_scr[2 * p + 1, 0:rows]])
        chunk_loop(compute, lambda p, e, o: put(p + 8, i, e, o), nxt)

    def layernorm(c0):
        xb = x_scr[:, pl.ds(c0, 128)].astype(f32)
        mu = jnp.mean(xb, axis=0, keepdims=True)
        xc = xb - mu
        var = jnp.mean(xc * xc, axis=0, keepdims=True)
        xn = (xc * jax.lax.rsqrt(var + 1e-5)).astype(bf16).astype(f32)
        xn = jnp.concatenate([xn, jnp.zeros((DP - D, 128), f32)], axis=0)
        xn_scr[pl.ds(c0, 128), :] = xn.T

    def ffn1(r0, h0, rows, n):
        f0, fn = _FCH[n]
        hid = _dot(xn_scr[pl.ds(r0, rows), 0:D], w1_raw[:, f0:f0 + fn])
        hh = 0.5 * hid
        hid_scr[pl.ds(h0, rows // 2), f0:f0 + fn] = _pack(hh * jnp.tanh(hh) + hh)

    wait(cx[0])
    layernorm(0)
    wait(cx[1], c1[0])
    for b in range(6):
        layernorm(128 * (b + 1))
        ffn1(128 * b, 64 * b, 128, 0)
    wait(c1[1], c1[2], c1[3])
    for n in range(1, 4):
        for b in range(6):
            ffn1(128 * b, 64 * b, 128, n)
    wait(ck[0], cq[0], cq[1], cq[2])
    m_rows(0, [ck[1], ck[2]])
    m_rows(1, None)
    m_rows(2, [cq[3], ck[3]])
    m_rows(3, [cv[0], co[0]])
    b_rows(0, [cv[1]])
    b_rows(1, [cv[2], cv[3], co[1]])
    b_rows(2, None)
    b_rows(3, [c2, cx[2]])

    lane = jax.lax.broadcasted_iota(jnp.int32, (L, 128), 1)
    row = jax.lax.broadcasted_iota(jnp.int32, (L, 128), 0)
    low = lane < 64

    def proj(h, idx):
        return _dot(h[:, 0:DM], _unpack(w_scr[idx]))

    def key_blocks(haug):
        rem = haug[:, 384:512]
        par = [jnp.where(low, rem, 0.0), jnp.where(low, 0.0, rem)]
        z = {}
        for t in range(5):
            for g in _GROUPS[t]:
                rows = []
                for hd, lo, hi in _PARTS[t]:
                    k0 = 128 * t + lo - 40 * hd
                    rows.append(par[hd % 2][k0:k0 + hi - lo] if hd in g else jnp.zeros((hi - lo, 128), f32))
                z[t, g] = jnp.concatenate(rows, axis=0).astype(bf16)
        return z

    def stacks(pr):
        rows = []
        for r in pr:
            rem = r[:, 768:896]
            rows.append(jnp.concatenate([r[:, 0:384], jnp.where(low, rem, 0.0)], axis=1))
            rows.append(jnp.concatenate([r[:, 384:768], jnp.where(low, 0.0, rem)], axis=1))
        return jnp.concatenate(rows, axis=0).astype(bf16)

    def softmax(sc):
        sg, masks = [], []
        for t in range(5):
            col = lane + 128 * t
            key = col
            for (j, lo, hi) in _PARTS[t]:
                key = jnp.where(lane >= lo, col - 40 * j, key)
            valid = (row < M) | (row >= key)
            sg.append(jnp.where(valid, sc[:, t * 128:(t + 1) * 128], -1e9))
            masks.append([(lane >= lo) & (lane < hi) for (_, lo, hi) in _PARTS[t]])

        def reduce(vals, op, fill, comb):
            red = [[op(jnp.where(mk, vals[t], fill), axis=1, keepdims=True) for mk in masks[t]] for t in range(5)]
            for t in range(4):
                both = comb(red[t][-1], red[t + 1][0])
                red[t][-1] = both
                red[t + 1][0] = both
            out = []
            for t in range(5):
                b = red[t][0]
                for n in range(1, len(red[t])):
                    b = jnp.where(lane >= _PARTS[t][n][1], red[t][n], b)
                out.append(b)
            return out
        mx = reduce(sg, jnp.max, -jnp.inf, jnp.maximum)
        e = [jnp.exp(sg[t] - mx[t]) for t in range(5)]
        l = reduce(e, jnp.sum, 0.0, jnp.add)
        ps = []
        for t in range(5):
            r = pl.reciprocal(l[t], approx=True)
            r = r * (2.0 - l[t] * r)
            ps.append(e[t] * r)
        return jnp.concatenate(ps, axis=1)

    def ffn2(blk, n):
        f0, fn = _FCH[n]
        hid = _unpack(hid_scr[pl.ds(pl.multiple_of(blk * 64, 64), 64), f0:f0 + fn])
        part = _dot(w2_raw[:, f0:f0 + fn], hid, NT)
        if n == 0:
            bt_scr[...] = part
        else:
            bt_scr[...] += part

    def filler(blk, g):
        stage, n = _FILL[g]
        if stage == 1:
            ffn1(pl.multiple_of(768 + 80 * blk, 8), pl.multiple_of(384 + 40 * blk, 8), 80, n)
        else:
            ffn2(blk, n)

    def step(blk, i, m):
        c0 = blk * 128
        xs = xn_scr[pl.ds(pl.multiple_of(c0 + i * SEG, SEG), SEG), :]
        h = jnp.concatenate([m, xs], axis=0)
        hr = h[:, 384:512]
        haug = jnp.concatenate([h[:, :384], hr + pltpu.roll(hr, 64, 1)], axis=1)
        z = key_blocks(haug)
        tall = stacks([proj(h, p) for p in range(8)])
        qr = _dot(h, _unpack(wq_scr[...]))
        upr = [proj(h, 8 + p) for p in range(NU0)]
        tt_scr[...] = pltpu.bitcast(tall.T, u32)
        sc = _dot(haug, _unpack(tt_scr[...]))
        for n, key in enumerate(z):
            zt_scr[n] = pltpu.bitcast(z[key].T, u32)

        def qpair(g):
            he, ho = qr[:, (g[0] // 2) * 128:(g[0] // 2 + 1) * 128], qr[:, (g[1] // 2) * 128:(g[1] // 2 + 1) * 128]
            return he if g[0] // 2 == g[1] // 2 else jnp.where(low, he, ho)
        zt = {key: _unpack(zt_scr[n]) for n, key in enumerate(z)}
        sc = sc + jnp.concatenate(
            [sum(_dot(qpair(g), zt[t, g]) for g in _GROUPS[t]) for t in range(5)], axis=1)
        upr += [proj(h, 8 + p) for p in range(NU0, 8)]
        pfull = softmax(sc)
        uall = stacks(upr)
        yp = {key: _dot(pfull[:, key[0] * 128:(key[0] + 1) * 128], z[key]) for key in z}
        yr = []
        for j in range(8):
            lo_keys = [k for k in z if k[1][0] == 2 * j]
            hi_keys = [k for k in z if k[1][1] == 2 * j + 1]
            lo_sum = sum(yp[k] for k in lo_keys)
            yr.append(lo_sum if lo_keys == hi_keys else jnp.where(low, lo_sum, sum(yp[k] for k in hi_keys)))
        yr = jnp.concatenate(yr, axis=1)
        filler(blk, 2 * i)
        last = i == UNROLL - 1 and TAILV
        o = _dot(pfull, uall)
        if last:
            filler(blk, 2 * i + 1)
        o = o + _dot(yr, _unpack(wb_scr[...]))
        if not last:
            filler(blk, 2 * i + 1)
        res_scr[i * SEG:(i + 1) * SEG, :] = o[M:L]
        return o[0:M]

    def emit(blk):
        c0 = pl.multiple_of(blk * 128, 128)
        rt = res_scr[...].T
        rt = jnp.concatenate([rt[0:384], rt[384:448] + rt[448:512]], axis=0)
        out_scr[blk] = (x_scr[:, pl.ds(c0, 128)].astype(f32) + rt + bt_scr[...]).astype(bf16)

    def out_dma(blk):
        c0 = pl.multiple_of(blk * 128, 128)
        return pltpu.make_async_copy(out_scr.at[blk], out_hbm.at[:, pl.ds(c0, 128)], osems.at[blk])

    def body(blk, m):
        emit(jnp.maximum(blk - 1, 0))
        for i in range(UNROLL):
            m = step(blk, i, m)
        layernorm(pl.multiple_of(jnp.minimum(blk + 7, NBLK - 1) * 128, 128))

        @pl.when(blk > 0)
        def _():
            out_dma(blk - 1).start()
        return m

    m0 = jnp.concatenate([mem_ref[...].astype(f32), jnp.zeros((M, DP - D), f32)], axis=1)
    jax.lax.fori_loop(0, NBLK, body, m0)
    emit(NBLK - 1)
    out_dma(NBLK - 1).start()
    for b in range(NBLK):
        out_dma(b).wait()


@jax.jit
def run(A_x, A_mem0, A_Wq, A_Wk, A_Wv, A_Wo, B_w1, B_w2):
    vm = pl.BlockSpec(memory_space=pltpu.VMEM)
    anyspec = pl.BlockSpec(memory_space=pl.ANY)
    out_t = pl.pallas_call(
        kernel,
        out_shape=jax.ShapeDtypeStruct((D, S), bf16),
        in_specs=[anyspec, vm, anyspec, anyspec, anyspec, anyspec, anyspec, anyspec],
        out_specs=anyspec,
        scratch_shapes=[
            pltpu.VMEM((2, D * H, 128), bf16),
            pltpu.VMEM((2, D * H, 128), bf16),
            pltpu.VMEM((2, D * H, 128), bf16),
            pltpu.VMEM((H, D, DH), bf16),
            pltpu.VMEM((D, S), bf16),
            pltpu.VMEM((D, F), bf16),
            pltpu.VMEM((D, F), bf16),
            pltpu.SemaphoreType.DMA((NSEM,)),
            pltpu.SemaphoreType.DMA((NBLK,)),
            pltpu.VMEM((16, DM // 2, 896), u32),
            pltpu.VMEM((DP // 2, 1024), u32),
            pltpu.VMEM((512, DP), u32),
            pltpu.VMEM((S, DP), f32),
            pltpu.VMEM((128, DP), f32),
            pltpu.VMEM((NBLK, D, 128), bf16),
            pltpu.VMEM((S // 2, F), u32),
            pltpu.VMEM((D, 128), f32),
            pltpu.VMEM((DP // 2, 640), u32),
            pltpu.VMEM((10, 64, 128), u32),
            pltpu.VMEM((H, DM // 2, DH), u32),
            pltpu.VMEM((H, DM // 2, DH), u32),
        ],
        compiler_params=pltpu.CompilerParams(vmem_limit_bytes=120 * 1024 * 1024),
    )(jnp.swapaxes(A_x, 1, 2).reshape(D, S), A_mem0.reshape(M, D), A_Wq.reshape(D * H, DH),
      A_Wk.reshape(D * H, DH), A_Wv.reshape(D * H, DH), jnp.swapaxes(A_Wo, 1, 2), B_w1, B_w2.T)
    return jnp.swapaxes(out_t.reshape(1, D, S), 1, 2)


def pallas_parallel_sum__memory_aug_recurrent_mem_tr__dense_activation_silu__prompt_kernel(A_x, A_mem0, A_Wq, A_Wk, A_Wv, A_Wo, A_seg_len, B_x, B_w1, B_w2):
    return run(A_x, A_mem0, A_Wq, A_Wk, A_Wv, A_Wo, B_w1, B_w2)
```

```python
import jax
import jax.numpy as jnp
from jax.experimental import pallas as pl
from jax.experimental.pallas import tpu as pltpu

S, D, H, DH, M, SEG, F = 2048, 448, 16, 256, 8, 32, 1792
L = M + SEG
DP = 512
DM = 384
BLK = 128
NBLK = S // BLK
PRE = 768
AHEAD = (S - PRE) // NBLK
f32, bf16, u32 = jnp.float32, jnp.bfloat16, jnp.uint32
NN = (((1,), (0,)), ((), ()))
NT = (((1,), (1,)), ((), ()))

PARTS = [[(j, max(L * j, 128 * t) - 128 * t, min(L * j + L, 128 * t + 128) - 128 * t)
          for j in range(H) if L * j < 128 * t + 128 and L * j + L > 128 * t] for t in range(5)]
GROUPS = [[tuple(sorted((p[i][0], p[i + 1][0]), key=lambda hd: hd % 2)) for i in (0, 2)] for p in PARTS]
FCH = [(0, 384), (384, 512), (896, 384), (1280, 512)]
FILL = [(1, 0), (1, 1), (1, 2), (2, 0), (1, 3), (2, 1), (2, 2), (2, 3)]
WCH = [(0, 128), (128, 128), (256, 128), (384, 64)]
NSEM = 34


def _dot(a, b, dims=NN):
    return jax.lax.dot_general(a, b, dims, preferred_element_type=f32)


def _pack(x):
    return pltpu.bitcast(x.astype(bf16), u32)


def _unpack(x):
    return pltpu.bitcast(x, bf16)


def _kernel(x_hbm, mem_ref, wq_hbm, wk_hbm, wv_hbm, wo_hbm, w1_hbm, w2_hbm, out_hbm,
            q_scr, k_scr, v_scr, wo_scr, x_scr, w1_scr, w2_scr, sems, osems,
            w_scr, wq_scr, wb_scr, xn_scr, res_scr, out_scr, hid_scr, bt_scr, tt_scr, zt_scr, qh_scr, kh_scr):
    nsem = [0]

    def copy(src, dst):
        nsem[0] += 1
        return pltpu.make_async_copy(src, dst, sems.at[nsem[0] - 1])

    def head_chunks(src, dst):
        return [[copy(src.at[pl.ds(r0 * H, n * H), pl.ds(c * 128, 128)], dst.at[c, pl.ds(r0 * H, n * H), :])
                 for c in range(2)] for r0, n in WCH]
    cq, ck, cv = head_chunks(wq_hbm, q_scr), head_chunks(wk_hbm, k_scr), head_chunks(wv_hbm, v_scr)
    co = [copy(wo_hbm.at[:, pl.ds(r0, n), :], wo_scr.at[:, pl.ds(r0, n), :]) for r0, n in ((0, DM), (DM, D - DM))]
    cx = [copy(x_hbm.at[:, pl.ds(a, b - a)], x_scr.at[:, pl.ds(a, b - a)])
          for a, b in ((0, BLK), (BLK, PRE + BLK), (PRE + BLK, S))]
    c1 = [copy(w1_hbm.at[:, pl.ds(f0, fn)], w1_scr.at[:, pl.ds(f0, fn)]) for f0, fn in FCH]
    c2 = copy(w2_hbm, w2_scr)
    assert nsem[0] == NSEM

    def start(*cs):
        for c in cs:
            for d in (c if isinstance(c, list) else [c]):
                d.start()

    def wait(*cs):
        for c in cs:
            for d in (c if isinstance(c, list) else [c]):
                d.wait()

    start(cx[0], cx[1], c1, ck[0], cq[0], cq[1], cq[2], ck[1], ck[2], cq[3], ck[3], cv[0], co[0],
          cv[1], cv[2], cv[3], co[1], c2, cx[2])
    res_scr[...] = jnp.zeros((BLK, DP), f32)
    bt_scr[...] = jnp.zeros((D, BLK), f32)

    def layernorm(c0):
        xb = x_scr[:, pl.ds(c0, BLK)].astype(f32)
        mu = jnp.mean(xb, axis=0, keepdims=True)
        xc = xb - mu
        var = jnp.mean(xc * xc, axis=0, keepdims=True)
        xn = (xc * jax.lax.rsqrt(var + 1e-5)).astype(bf16).astype(f32)
        xn = jnp.concatenate([xn, jnp.zeros((DP - D, BLK), f32)], axis=0)
        xn_scr[pl.ds(c0, BLK), :] = xn.T

    def dense1(r0, h0, rows, n):
        f0, fn = FCH[n]
        hid = _dot(xn_scr[pl.ds(r0, rows), 0:D], w1_scr[:, f0:f0 + fn])
        hh = 0.5 * hid
        hid_scr[pl.ds(h0, rows // 2), f0:f0 + fn] = _pack(hh * jnp.tanh(hh) + hh)

    def dense2(blk, n):
        f0, fn = FCH[n]
        hid = _unpack(hid_scr[pl.ds(pl.multiple_of(blk * (BLK // 2), BLK // 2), BLK // 2), f0:f0 + fn])
        part = _dot(w2_scr[:, f0:f0 + fn], hid, NT)
        if n == 0:
            bt_scr[...] = part
        else:
            bt_scr[...] += part

    def heads(scr, p, r0, n, mul=None):
        los, his = [], []
        for c in range(2):
            w = scr.at[c].bitcast(u32)[pl.ds(p + 8 * r0, n, stride=8), :]
            los.append(pltpu.bitcast(w << 16, f32))
            his.append(pltpu.bitcast(w & jnp.uint32(0xffff0000), f32))
        lo, hi = jnp.concatenate(los, axis=1), jnp.concatenate(his, axis=1)
        return (lo, hi) if mul is None else (lo * mul, hi * mul)

    def fold(i, p, lhs, rhs):
        rows = lhs(128 * i, WCH[i][1])

        def one(par):
            if i < 3:
                kh_scr[2 * p + par, 64 * i:64 * (i + 1), :] = _pack(rows[par])
                return _dot(rows[par], rhs[par][0:DM], NT)
            return (_dot(rows[par], rhs[par], NT),
                    _dot(rhs[par][DM:D], _unpack(kh_scr[2 * p + par]), NT))
        return one(0), one(1)

    def store(idx, i, e, o):
        if i < 3:
            w_scr[idx, 64 * i:64 * (i + 1), 0:2 * DM] = jnp.concatenate([_pack(e), _pack(o)], axis=1)
            return
        w_scr[idx, :, 2 * DM:2 * DM + 128] = _pack(jnp.concatenate([e[1], o[1]], axis=0).T)
        t = jnp.concatenate([e[0], o[0]], axis=0)
        if idx < 8:
            wq_scr[:, idx * 128:(idx + 1) * 128] = _pack(jnp.concatenate([t, t[:, DM:D]], axis=1).T)
        else:
            wb_scr[(idx - 8) * 64:(idx - 7) * 64, :] = _pack(
                jnp.concatenate([t, jnp.zeros((128, DP - D), f32)], axis=1))

    def fold_chunk(compute, idx0, i, nxt):
        for p in range(8):
            e, o = compute(p)
            if p == 7 and nxt:
                wait(*nxt)
            store(idx0 + p, i, e, o)

    def m_chunk(i, nxt):
        def compute(p):
            if i == 0:
                q = [t.astype(bf16) for t in heads(q_scr, p, 0, DM)]
                qh_scr[2 * p] = pltpu.bitcast(q[0], u32)
                qh_scr[2 * p + 1] = pltpu.bitcast(q[1], u32)
            else:
                q = [_unpack(qh_scr[2 * p]), _unpack(qh_scr[2 * p + 1])]
            if i == 3:
                q = [jnp.concatenate([a, b.astype(bf16)], axis=0) for a, b in zip(q, heads(q_scr, p, DM, D - DM))]
            return fold(i, p, lambda r0, n: heads(k_scr, p, r0, n, DH ** -0.5), q)
        fold_chunk(compute, 0, i, nxt)

    def b_chunk(i, nxt):
        def compute(p):
            rows = D if i == 3 else DM
            return fold(i, p, lambda r0, n: heads(v_scr, p, r0, n),
                        [wo_scr[2 * p, 0:rows], wo_scr[2 * p + 1, 0:rows]])
        fold_chunk(compute, 8, i, nxt)

    wait(cx[0])
    layernorm(0)
    wait(cx[1], c1[0])
    for b in range(PRE // BLK):
        layernorm(BLK * (b + 1))
        dense1(BLK * b, BLK // 2 * b, BLK, 0)
    wait(c1[1], c1[2], c1[3])
    for n in range(1, 4):
        for b in range(PRE // BLK):
            dense1(BLK * b, BLK // 2 * b, BLK, n)
    wait(ck[0], cq[0], cq[1], cq[2])
    m_chunk(0, [ck[1], ck[2]])
    m_chunk(1, None)
    m_chunk(2, [cq[3], ck[3]])
    m_chunk(3, [cv[0], co[0]])
    b_chunk(0, [cv[1]])
    b_chunk(1, [cv[2], cv[3], co[1]])
    b_chunk(2, None)
    b_chunk(3, [c2, cx[2]])

    lane = jax.lax.broadcasted_iota(jnp.int32, (L, 128), 1)
    row = jax.lax.broadcasted_iota(jnp.int32, (L, 128), 0)
    low = lane < 64

    def project(h, idx):
        return _dot(h[:, 0:DM], _unpack(w_scr[idx]))

    def stack(pairs):
        rows = []
        for r in pairs:
            rem = r[:, 2 * DM:2 * DM + 128]
            rows.append(jnp.concatenate([r[:, 0:DM], jnp.where(low, rem, 0.0)], axis=1))
            rows.append(jnp.concatenate([r[:, DM:2 * DM], jnp.where(low, 0.0, rem)], axis=1))
        return jnp.concatenate(rows, axis=0).astype(bf16)

    def key_remainders(haug):
        rem = haug[:, DM:DP]
        par = [jnp.where(low, rem, 0.0), jnp.where(low, 0.0, rem)]
        z = {}
        for t in range(5):
            for g in GROUPS[t]:
                rows = []
                for hd, lo, hi in PARTS[t]:
                    k0 = 128 * t + lo - L * hd
                    rows.append(par[hd % 2][k0:k0 + hi - lo] if hd in g else jnp.zeros((hi - lo, 128), f32))
                z[t, g] = jnp.concatenate(rows, axis=0).astype(bf16)
        return z

    def softmax(sc):
        sg, masks = [], []
        for t in range(5):
            col = lane + 128 * t
            key = col
            for j, lo, _ in PARTS[t]:
                key = jnp.where(lane >= lo, col - L * j, key)
            valid = (row < M) | (row >= key)
            sg.append(jnp.where(valid, sc[:, t * 128:(t + 1) * 128], -1e9))
            masks.append([(lane >= lo) & (lane < hi) for _, lo, hi in PARTS[t]])

        def per_head(vals, op, fill, comb):
            red = [[op(jnp.where(mk, vals[t], fill), axis=1, keepdims=True) for mk in masks[t]] for t in range(5)]
            for t in range(4):
                both = comb(red[t][-1], red[t + 1][0])
                red[t][-1] = both
                red[t + 1][0] = both
            out = []
            for t in range(5):
                b = red[t][0]
                for n in range(1, len(red[t])):
                    b = jnp.where(lane >= PARTS[t][n][1], red[t][n], b)
                out.append(b)
            return out
        mx = per_head(sg, jnp.max, -jnp.inf, jnp.maximum)
        e = [jnp.exp(sg[t] - mx[t]) for t in range(5)]
        den = per_head(e, jnp.sum, 0.0, jnp.add)
        ps = []
        for t in range(5):
            r = pl.reciprocal(den[t], approx=True)
            r = r * (2.0 - den[t] * r)
            ps.append(e[t] * r)
        return jnp.concatenate(ps, axis=1)

    def fill(blk, g):
        layer, n = FILL[g]
        if layer == 1:
            dense1(pl.multiple_of(PRE + AHEAD * blk, 8), pl.multiple_of(PRE // 2 + AHEAD // 2 * blk, 8), AHEAD, n)
        else:
            dense2(blk, n)

    def step(blk, i, m):
        xs = xn_scr[pl.ds(pl.multiple_of(blk * BLK + i * SEG, SEG), SEG), :]
        h = jnp.concatenate([m, xs], axis=0)
        hr = h[:, DM:DP]
        haug = jnp.concatenate([h[:, :DM], hr + pltpu.roll(hr, 64, 1)], axis=1)
        z = key_remainders(haug)
        keys = stack([project(h, p) for p in range(8)])
        qr = _dot(h, _unpack(wq_scr[...]))
        vals = [project(h, 8 + p) for p in range(3)]
        tt_scr[...] = pltpu.bitcast(keys.T, u32)
        sc = _dot(haug, _unpack(tt_scr[...]))
        for n, key in enumerate(z):
            zt_scr[n] = pltpu.bitcast(z[key].T, u32)
        zt = {key: _unpack(zt_scr[n]) for n, key in enumerate(z)}

        def qgroup(g):
            ev, od = (qr[:, (hd // 2) * 128:(hd // 2 + 1) * 128] for hd in g)
            return ev if g[0] // 2 == g[1] // 2 else jnp.where(low, ev, od)
        sc = sc + jnp.concatenate(
            [sum(_dot(qgroup(g), zt[t, g]) for g in GROUPS[t]) for t in range(5)], axis=1)
        vals += [project(h, 8 + p) for p in range(3, 8)]
        p_all = softmax(sc)
        v_all = stack(vals)
        part = {key: _dot(p_all[:, key[0] * 128:(key[0] + 1) * 128], z[key]) for key in z}
        yr = []
        for j in range(8):
            lo_keys = [k for k in z if k[1][0] == 2 * j]
            hi_keys = [k for k in z if k[1][1] == 2 * j + 1]
            lo_sum = sum(part[k] for k in lo_keys)
            yr.append(lo_sum if lo_keys == hi_keys else jnp.where(low, lo_sum, sum(part[k] for k in hi_keys)))
        yr = jnp.concatenate(yr, axis=1)
        fill(blk, 2 * i)
        last = i == BLK // SEG - 1
        o = _dot(p_all, v_all)
        if last:
            fill(blk, 2 * i + 1)
        o = o + _dot(yr, _unpack(wb_scr[...]))
        if not last:
            fill(blk, 2 * i + 1)
        res_scr[i * SEG:(i + 1) * SEG, :] = o[M:L]
        return o[0:M]

    def emit(blk):
        c0 = pl.multiple_of(blk * BLK, BLK)
        rt = res_scr[...].T
        rt = jnp.concatenate([rt[0:DM], rt[DM:D] + rt[D:DP]], axis=0)
        out_scr[blk] = (x_scr[:, pl.ds(c0, BLK)].astype(f32) + rt + bt_scr[...]).astype(bf16)

    def out_copy(blk):
        c0 = pl.multiple_of(blk * BLK, BLK)
        return pltpu.make_async_copy(out_scr.at[blk], out_hbm.at[:, pl.ds(c0, BLK)], osems.at[blk])

    def body(blk, m):
        emit(jnp.maximum(blk - 1, 0))
        for i in range(BLK // SEG):
            m = step(blk, i, m)
        layernorm(pl.multiple_of(jnp.minimum(blk + PRE // BLK + 1, NBLK - 1) * BLK, BLK))

        @pl.when(blk > 0)
        def _():
            out_copy(blk - 1).start()
        return m

    m0 = jnp.concatenate([mem_ref[...].astype(f32), jnp.zeros((M, DP - D), f32)], axis=1)
    jax.lax.fori_loop(0, NBLK, body, m0)
    emit(NBLK - 1)
    out_copy(NBLK - 1).start()
    for b in range(NBLK):
        out_copy(b).wait()


@jax.jit
def _run(A_x, A_mem0, A_Wq, A_Wk, A_Wv, A_Wo, B_w1, B_w2):
    hbm = pl.BlockSpec(memory_space=pl.ANY)
    out_t = pl.pallas_call(
        _kernel,
        out_shape=jax.ShapeDtypeStruct((D, S), bf16),
        in_specs=[hbm, pl.BlockSpec(memory_space=pltpu.VMEM), hbm, hbm, hbm, hbm, hbm, hbm],
        out_specs=hbm,
        scratch_shapes=[
            pltpu.VMEM((2, D * H, 128), bf16),
            pltpu.VMEM((2, D * H, 128), bf16),
            pltpu.VMEM((2, D * H, 128), bf16),
            pltpu.VMEM((H, D, DH), bf16),
            pltpu.VMEM((D, S), bf16),
            pltpu.VMEM((D, F), bf16),
            pltpu.VMEM((D, F), bf16),
            pltpu.SemaphoreType.DMA((NSEM,)),
            pltpu.SemaphoreType.DMA((NBLK,)),
            pltpu.VMEM((16, DM // 2, 896), u32),
            pltpu.VMEM((DP // 2, 1024), u32),
            pltpu.VMEM((512, DP), u32),
            pltpu.VMEM((S, DP), f32),
            pltpu.VMEM((BLK, DP), f32),
            pltpu.VMEM((NBLK, D, BLK), bf16),
            pltpu.VMEM((S // 2, F), u32),
            pltpu.VMEM((D, BLK), f32),
            pltpu.VMEM((DP // 2, 640), u32),
            pltpu.VMEM((10, 64, 128), u32),
            pltpu.VMEM((H, DM // 2, DH), u32),
            pltpu.VMEM((H, DM // 2, DH), u32),
        ],
        compiler_params=pltpu.CompilerParams(vmem_limit_bytes=120 * 1024 * 1024),
    )(jnp.swapaxes(A_x, 1, 2).reshape(D, S), A_mem0.reshape(M, D), A_Wq.reshape(D * H, DH),
      A_Wk.reshape(D * H, DH), A_Wv.reshape(D * H, DH), jnp.swapaxes(A_Wo, 1, 2), B_w1, B_w2.T)
    return jnp.swapaxes(out_t.reshape(1, D, S), 1, 2)


def pallas_parallel_sum__memory_aug_recurrent_mem_tr__dense_activation_silu__prompt_kernel(
        A_x, A_mem0, A_Wq, A_Wk, A_Wv, A_Wo, A_seg_len, B_x, B_w1, B_w2):
    return _run(A_x, A_mem0, A_Wq, A_Wk, A_Wv, A_Wo, B_w1, B_w2)
```

```python
import jax
import jax.numpy as jnp
from jax.experimental import pallas as pl
from jax.experimental.pallas import tpu as pltpu

S, D, H, DH, M, SEG, F = 2048, 448, 16, 256, 8, 32, 1792
L = M + SEG
DP = 512
DM = 384
BLK = 128
NBLK = S // BLK
PRE = 1024
AHEAD = (S - PRE) // NBLK
f32, bf16, u32 = jnp.float32, jnp.bfloat16, jnp.uint32
NN = (((1,), (0,)), ((), ()))
NT = (((1,), (1,)), ((), ()))

PARTS = [[(j, max(L * j, 128 * t) - 128 * t, min(L * j + L, 128 * t + 128) - 128 * t)
          for j in range(H) if L * j < 128 * t + 128 and L * j + L > 128 * t] for t in range(5)]
GROUPS = [[tuple(sorted((p[i][0], p[i + 1][0]), key=lambda hd: hd % 2)) for i in (0, 2)] for p in PARTS]
FCH = [(0, 384), (384, 512), (896, 384), (1280, 512)]
FILL = [(1, 0), (1, 1), (1, 2), (2, 0), (2, 1), (1, 3), (2, 2), (2, 3)]
WCH = [(0, 128), (128, 128), (256, 128), (384, 64)]
NSEM = 44


def _dot(a, b, dims=NN):
    return jax.lax.dot_general(a, b, dims, preferred_element_type=f32)


def _pack(x):
    return pltpu.bitcast(x.astype(bf16), u32)


def _unpack(x):
    return pltpu.bitcast(x, bf16)


def _kernel(x_hbm, mem_ref, wq_hbm, wk_hbm, wv_hbm, wo_hbm, w1_hbm, w2_hbm, out_hbm,
            q_scr, k_scr, v_scr, wo_scr, x_scr, w1_scr, w2_scr, sems, osems,
            w_scr, wq_scr, wb_scr, xn_scr, res_scr, out_scr, hid_scr, bt_scr, tt_scr, zt_scr, qh_scr, kh_scr):
    nsem = [0]

    def copy(src, dst):
        nsem[0] += 1
        return pltpu.make_async_copy(src, dst, sems.at[nsem[0] - 1])

    def head_chunks(src, dst):
        return [[copy(src.at[pl.ds(r0 * H, n * H), pl.ds(c * 128, 128)], dst.at[c, pl.ds(r0 * H, n * H), :])
                 for c in range(2)] for r0, n in WCH]
    cq, ck, cv = head_chunks(wq_hbm, q_scr), head_chunks(wk_hbm, k_scr), head_chunks(wv_hbm, v_scr)
    co = [copy(wo_hbm.at[:, pl.ds(r0, n), :], wo_scr.at[:, pl.ds(r0, n), :]) for r0, n in ((0, DM), (DM, D - DM))]
    xcols = [(BLK * b, BLK) for b in range(PRE // BLK + 1)] + [(PRE + BLK, S - PRE - BLK)]
    cx = [copy(x_hbm.at[:, pl.ds(a, n)], x_scr.at[:, pl.ds(a, n)]) for a, n in xcols]
    c1 = [copy(w1_hbm.at[:, pl.ds(f0, fn)], w1_scr.at[:, pl.ds(f0, fn)]) for f0, fn in FCH]
    c2 = copy(w2_hbm, w2_scr)
    pin1 = copy(w1_hbm.at[:, pl.ds(0, 128)], w1_scr.at[:, pl.ds(F, 128)])
    pin2 = copy(wk_hbm.at[pl.ds(0, 16), pl.ds(0, 128)], k_scr.at[0, pl.ds(D * H, 16), :])
    pin3 = copy(wv_hbm.at[pl.ds(0, 16), pl.ds(0, 128)], v_scr.at[0, pl.ds(D * H, 16), :])
    assert nsem[0] == NSEM

    def start(*cs):
        for c in cs:
            for d in (c if isinstance(c, list) else [c]):
                d.start()

    def wait(*cs):
        for c in cs:
            for d in (c if isinstance(c, list) else [c]):
                d.wait()

    start(cx[0], c1[0], cx[1:-1], c1[1:], pin1, pin2, pin3, ck[0], cq[0], cq[1], cq[2], ck[1], ck[2],
          ck[3], cq[3], cv[0], co[0], cv[1], cv[2], cv[3], co[1], c2, cx[-1])
    res_scr[...] = jnp.zeros((BLK, DP), f32)
    bt_scr[...] = jnp.zeros((D, BLK), f32)

    def layernorm(c0):
        xb = x_scr[:, pl.ds(c0, BLK)].astype(f32)
        mu = jnp.mean(xb, axis=0, keepdims=True)
        xc = xb - mu
        var = jnp.mean(xc * xc, axis=0, keepdims=True)
        xn = (xc * jax.lax.rsqrt(var + 1e-5)).astype(bf16).astype(f32)
        xn = jnp.concatenate([xn, jnp.zeros((DP - D, BLK), f32)], axis=0)
        xn_scr[pl.ds(c0, BLK), :] = xn.T

    def dense1(r0, h0, rows, n):
        f0, fn = FCH[n]
        hid = _dot(xn_scr[pl.ds(r0, rows), 0:D], w1_scr[:, f0:f0 + fn])
        hh = 0.5 * hid
        hid_scr[pl.ds(h0, rows // 2), f0:f0 + fn] = _pack(hh * jnp.tanh(hh) + hh)

    def dense2(blk, n):
        f0, fn = FCH[n]
        hid = _unpack(hid_scr[pl.ds(pl.multiple_of(blk * (BLK // 2), BLK // 2), BLK // 2), f0:f0 + fn])
        part = _dot(w2_scr[:, f0:f0 + fn], hid, NT)
        if n == 0:
            bt_scr[...] = part
        else:
            bt_scr[...] += part

    def heads(scr, p, r0, n, mul=None):
        los, his = [], []
        for c in range(2):
            w = scr.at[c].bitcast(u32)[pl.ds(p + 8 * r0, n, stride=8), :]
            los.append(pltpu.bitcast(w << 16, f32))
            his.append(pltpu.bitcast(w & jnp.uint32(0xffff0000), f32))
        lo, hi = jnp.concatenate(los, axis=1), jnp.concatenate(his, axis=1)
        return (lo, hi) if mul is None else (lo * mul, hi * mul)

    def fold(i, p, lhs, rhs):
        rows = lhs(128 * i, WCH[i][1])

        def one(par):
            if i < 3:
                kh_scr[2 * p + par, 64 * i:64 * (i + 1), :] = _pack(rows[par])
                return _dot(rows[par], rhs[par][0:DM], NT)
            return (_dot(rows[par], rhs[par], NT),
                    _dot(rhs[par][DM:D], _unpack(kh_scr[2 * p + par]), NT))
        return one(0), one(1)

    def store(idx, i, e, o):
        if i < 3:
            w_scr[idx, 64 * i:64 * (i + 1), 0:2 * DM] = jnp.concatenate([_pack(e), _pack(o)], axis=1)
            return
        w_scr[idx, :, 2 * DM:2 * DM + 128] = _pack(jnp.concatenate([e[1], o[1]], axis=0).T)
        t = jnp.concatenate([e[0], o[0]], axis=0)
        if idx < 8:
            wq_scr[:, idx * 128:(idx + 1) * 128] = _pack(jnp.concatenate([t, t[:, DM:D]], axis=1).T)
        else:
            wb_scr[(idx - 8) * 64:(idx - 7) * 64, :] = _pack(
                jnp.concatenate([t, jnp.zeros((128, DP - D), f32)], axis=1))

    def fold_chunk(compute, idx0, i, nxt):
        for p in range(8):
            e, o = compute(p)
            store(idx0 + p, i, e, o)
        if nxt:
            wait(*nxt)

    def m_chunk(i, nxt):
        def compute(p):
            if i == 0:
                q = [t.astype(bf16) for t in heads(q_scr, p, 0, DM)]
                qh_scr[2 * p] = pltpu.bitcast(q[0], u32)
                qh_scr[2 * p + 1] = pltpu.bitcast(q[1], u32)
            else:
                q = [_unpack(qh_scr[2 * p]), _unpack(qh_scr[2 * p + 1])]
            if i == 3:
                q = [jnp.concatenate([a, b.astype(bf16)], axis=0) for a, b in zip(q, heads(q_scr, p, DM, D - DM))]
            return fold(i, p, lambda r0, n: heads(k_scr, p, r0, n, DH ** -0.5), q)
        fold_chunk(compute, 0, i, nxt)

    def b_chunk(i, nxt):
        def compute(p):
            rows = D if i == 3 else DM
            return fold(i, p, lambda r0, n: heads(v_scr, p, r0, n),
                        [wo_scr[2 * p, 0:rows], wo_scr[2 * p + 1, 0:rows]])
        fold_chunk(compute, 8, i, nxt)

    wait(cx[0])
    layernorm(0)
    wait(c1[0])
    for b in range(PRE // BLK):
        wait(cx[b + 1])
        layernorm(BLK * (b + 1))
        dense1(BLK * b, BLK // 2 * b, BLK, 0)
    wait(c1[1], c1[2], c1[3])
    for n in range(1, 4):
        for b in range(PRE // BLK):
            dense1(BLK * b, BLK // 2 * b, BLK, n)
    wait(pin1, ck[0], cq[0], cq[1], cq[2])
    m_chunk(0, [ck[1]])
    m_chunk(1, [ck[2]])
    m_chunk(2, [ck[3], cq[3]])
    m_chunk(3, [pin2, cv[0], co[0]])
    b_chunk(0, [cv[1]])
    b_chunk(1, [cv[2]])
    b_chunk(2, [cv[3], co[1]])
    b_chunk(3, [pin3, c2, cx[-1]])

    lane = jax.lax.broadcasted_iota(jnp.int32, (L, 128), 1)
    row = jax.lax.broadcasted_iota(jnp.int32, (L, 128), 0)
    low = lane < 64

    def project(h, idx):
        return _dot(h[:, 0:DM], _unpack(w_scr[idx]))

    def stack(pairs):
        rows = []
        for r in pairs:
            rem = r[:, 2 * DM:2 * DM + 128]
            rows.append(jnp.concatenate([r[:, 0:DM], jnp.where(low, rem, 0.0)], axis=1))
            rows.append(jnp.concatenate([r[:, DM:2 * DM], jnp.where(low, 0.0, rem)], axis=1))
        return jnp.concatenate(rows, axis=0).astype(bf16)

    def key_remainders(haug):
        rem = haug[:, DM:DP]
        par = [jnp.where(low, rem, 0.0), jnp.where(low, 0.0, rem)]
        z = {}
        for t in range(5):
            for g in GROUPS[t]:
                rows = []
                for hd, lo, hi in PARTS[t]:
                    k0 = 128 * t + lo - L * hd
                    rows.append(par[hd % 2][k0:k0 + hi - lo] if hd in g else jnp.zeros((hi - lo, 128), f32))
                z[t, g] = jnp.concatenate(rows, axis=0).astype(bf16)
        return z

    def softmax(sc):
        sg, masks = [], []
        for t in range(5):
            col = lane + 128 * t
            key = col
            for j, lo, _ in PARTS[t]:
                key = jnp.where(lane >= lo, col - L * j, key)
            valid = (row < M) | (row >= key)
            sg.append(jnp.where(valid, sc[:, t * 128:(t + 1) * 128], -1e9))
            masks.append([(lane >= lo) & (lane < hi) for _, lo, hi in PARTS[t]])

        def per_head(vals, op, fill, comb):
            red = [[op(jnp.where(mk, vals[t], fill), axis=1, keepdims=True) for mk in masks[t]] for t in range(5)]
            for t in range(4):
                both = comb(red[t][-1], red[t + 1][0])
                red[t][-1] = both
                red[t + 1][0] = both
            out = []
            for t in range(5):
                b = red[t][0]
                for n in range(1, len(red[t])):
                    b = jnp.where(lane >= PARTS[t][n][1], red[t][n], b)
                out.append(b)
            return out
        mx = per_head(sg, jnp.max, -jnp.inf, jnp.maximum)
        e = [jnp.exp(sg[t] - mx[t]) for t in range(5)]
        den = per_head(e, jnp.sum, 0.0, jnp.add)
        ps = []
        for t in range(5):
            r = pl.reciprocal(den[t], approx=True)
            r = r * (2.0 - den[t] * r)
            ps.append(e[t] * r)
        return jnp.concatenate(ps, axis=1)

    def fill(blk, g):
        layer, n = FILL[g]
        if layer == 1:
            dense1(pl.multiple_of(PRE + AHEAD * blk, 8), pl.multiple_of(PRE // 2 + AHEAD // 2 * blk, 8), AHEAD, n)
        else:
            dense2(blk, n)

    def step(blk, i, m):
        xs = xn_scr[pl.ds(pl.multiple_of(blk * BLK + i * SEG, SEG), SEG), :]
        h = jnp.concatenate([m, xs], axis=0)
        hr = h[:, DM:DP]
        haug = jnp.concatenate([h[:, :DM], hr + pltpu.roll(hr, 64, 1)], axis=1)
        z = key_remainders(haug)
        keys = stack([project(h, p) for p in range(8)])
        qr = _dot(h, _unpack(wq_scr[...]))
        vals = [project(h, 8 + p) for p in range(4)]
        tt_scr[...] = pltpu.bitcast(keys.T, u32)
        sc = _dot(haug, _unpack(tt_scr[...]))
        for n, key in enumerate(z):
            zt_scr[n] = pltpu.bitcast(z[key].T, u32)
        zt = {key: _unpack(zt_scr[n]) for n, key in enumerate(z)}

        def qgroup(g):
            ev, od = (qr[:, (hd // 2) * 128:(hd // 2 + 1) * 128] for hd in g)
            return ev if g[0] // 2 == g[1] // 2 else jnp.where(low, ev, od)
        sc = sc + jnp.concatenate(
            [sum(_dot(qgroup(g), zt[t, g]) for g in GROUPS[t]) for t in range(5)], axis=1)
        vals += [project(h, 8 + p) for p in range(4, 8)]
        p_all = softmax(sc)
        v_all = stack(vals)
        part = {key: _dot(p_all[:, key[0] * 128:(key[0] + 1) * 128], z[key]) for key in z}
        yr = []
        for j in range(8):
            lo_keys = [k for k in z if k[1][0] == 2 * j]
            hi_keys = [k for k in z if k[1][1] == 2 * j + 1]
            lo_sum = sum(part[k] for k in lo_keys)
            yr.append(lo_sum if lo_keys == hi_keys else jnp.where(low, lo_sum, sum(part[k] for k in hi_keys)))
        yr = jnp.concatenate(yr, axis=1)
        fill(blk, 2 * i)
        last = i == BLK // SEG - 1
        o = _dot(p_all, v_all)
        if last:
            fill(blk, 2 * i + 1)
        o = o + _dot(yr, _unpack(wb_scr[...]))
        if not last:
            fill(blk, 2 * i + 1)
        res_scr[i * SEG:(i + 1) * SEG, :] = o[M:L]
        return o[0:M]

    def emit(blk):
        c0 = pl.multiple_of(blk * BLK, BLK)
        rt = res_scr[...].T
        rt = jnp.concatenate([rt[0:DM], rt[DM:D] + rt[D:DP]], axis=0)
        out_scr[blk] = (x_scr[:, pl.ds(c0, BLK)].astype(f32) + rt + bt_scr[...]).astype(bf16)

    def out_copy(blk):
        c0 = pl.multiple_of(blk * BLK, BLK)
        return pltpu.make_async_copy(out_scr.at[blk], out_hbm.at[:, pl.ds(c0, BLK)], osems.at[blk])

    def body(blk, m):
        emit(jnp.maximum(blk - 1, 0))
        for i in range(BLK // SEG):
            m = step(blk, i, m)
        layernorm(pl.multiple_of(jnp.minimum(blk + PRE // BLK + 1, NBLK - 1) * BLK, BLK))

        @pl.when(blk > 0)
        def _():
            out_copy(blk - 1).start()
        return m

    m0 = jnp.concatenate([mem_ref[...].astype(f32), jnp.zeros((M, DP - D), f32)], axis=1)
    jax.lax.fori_loop(0, NBLK, body, m0)
    emit(NBLK - 1)
    out_copy(NBLK - 1).start()
    for b in range(NBLK):
        out_copy(b).wait()


@jax.jit
def _run(A_x, A_mem0, A_Wq, A_Wk, A_Wv, A_Wo, B_w1, B_w2):
    hbm = pl.BlockSpec(memory_space=pl.ANY)
    out_t = pl.pallas_call(
        _kernel,
        out_shape=jax.ShapeDtypeStruct((D, S), bf16),
        in_specs=[hbm, pl.BlockSpec(memory_space=pltpu.VMEM), hbm, hbm, hbm, hbm, hbm, hbm],
        out_specs=hbm,
        scratch_shapes=[
            pltpu.VMEM((2, D * H, 128), bf16),
            pltpu.VMEM((2, D * H + 16, 128), bf16),
            pltpu.VMEM((2, D * H + 16, 128), bf16),
            pltpu.VMEM((H, D, DH), bf16),
            pltpu.VMEM((D, S), bf16),
            pltpu.VMEM((D, F + 128), bf16),
            pltpu.VMEM((D, F), bf16),
            pltpu.SemaphoreType.DMA((NSEM,)),
            pltpu.SemaphoreType.DMA((NBLK,)),
            pltpu.VMEM((16, DM // 2, 896), u32),
            pltpu.VMEM((DP // 2, 1024), u32),
            pltpu.VMEM((512, DP), u32),
            pltpu.VMEM((S, DP), f32),
            pltpu.VMEM((BLK, DP), f32),
            pltpu.VMEM((NBLK, D, BLK), bf16),
            pltpu.VMEM((S // 2, F), u32),
            pltpu.VMEM((D, BLK), f32),
            pltpu.VMEM((DP // 2, 640), u32),
            pltpu.VMEM((10, 64, 128), u32),
            pltpu.VMEM((H, DM // 2, DH), u32),
            pltpu.VMEM((H, DM // 2, DH), u32),
        ],
        compiler_params=pltpu.CompilerParams(
            vmem_limit_bytes=120 * 1024 * 1024,
            flags={"XLA_TPU_RESCHEDULE_DMA_DONES": True}),
    )(jnp.swapaxes(A_x, 1, 2).reshape(D, S), A_mem0.reshape(M, D), A_Wq.reshape(D * H, DH),
      A_Wk.reshape(D * H, DH), A_Wv.reshape(D * H, DH), jnp.swapaxes(A_Wo, 1, 2), B_w1, B_w2.T)
    return jnp.swapaxes(out_t.reshape(1, D, S), 1, 2)


def pallas_parallel_sum__memory_aug_recurrent_mem_tr__dense_activation_silu__prompt_kernel(
        A_x, A_mem0, A_Wq, A_Wk, A_Wv, A_Wo, A_seg_len, B_x, B_w1, B_w2):
    return _run(A_x, A_mem0, A_Wq, A_Wk, A_Wv, A_Wo, B_w1, B_w2)
```
